```python
import os as _os
_os.environ.setdefault('JAX_PLATFORMS', 'cpu')
import jax
import jax.numpy as jnp

def _softmax(x, axis=-1):
    return jax.nn.softmax(x, axis=axis)

def _gelu(x):
    return jax.nn.gelu(x, approximate=True)

def _silu(x):
    return jax.nn.silu(x)

def _sigmoid(x):
    return jax.nn.sigmoid(x)

def _layernorm(x, axis=-1, eps=1e-05):
    m = jnp.mean(x, axis=axis, keepdims=True)
    v = jnp.var(x, axis=axis, keepdims=True)
    return (x - m) / jnp.sqrt(v + eps)

def _scatter_add(tgt, idx, src, axis=0):
    return tgt.at[idx].add(src)

def _segment_sum(src, seg, n):
    return jax.ops.segment_sum(src, seg, n)

class _Rng:

    def __init__(self, key):
        self._k = key

    def _next(self):
        self._k, sub = jax.random.split(self._k)
        return sub

    def normal(self, shape):
        return jax.random.normal(self._next(), shape, dtype=jnp.bfloat16)

    def randint(self, lo, hi, shape):
        return jax.random.randint(self._next(), shape, lo, hi, dtype=jnp.int32)

    def uniform(self, shape, lo=0.0, hi=1.0):
        return jax.random.uniform(self._next(), shape, jnp.bfloat16, lo, hi)

    def permutation(self, n):
        return jax.random.permutation(self._next(), n)
kernel_name = 'adaLN_cond__compressed_kv_cla__moe_arch_mod__prompt'

def setup_inputs():
    _rng = _Rng(jax.random.key(int.from_bytes(__import__("os").urandom(4), "little")))
    _w = lambda a: (lambda t: t.astype(jnp.bfloat16) if jnp.issubdtype(t.dtype, jnp.floating) else t)(jnp.asarray(a))

    def _A_setup():
        B, H, Sq, Sk, D, M = (1, 32, 2048, 2048, 128, 640)
        Dc = 4 * D
        return {'x': _w((lambda *s: _rng.normal(s) * 0.1)(B, Sq, M)), 'c_kv': _w((lambda *s: _rng.normal(s) * 0.8)(B, Sk, Dc)), 'w_q': _w((lambda *s: _rng.normal(s) * 1.6)(M, H, D) * M ** (-0.5)), 'w_uk': _w((lambda *s: _rng.normal(s) * 1.6)(Dc, H, D) * Dc ** (-0.5)), 'w_uv': _w((lambda *s: _rng.normal(s) * 0.8)(Dc, H, D) * Dc ** (-0.5)), 'w_o': _w((lambda *s: _rng.normal(s) * 0.8)(H, D, M) * (H * D) ** (-0.5))}
    _A_in = _A_setup()

    def _B_setup():
        B, S, D, F, C = (1, 2048, 640, 1728, 8)
        return {'x': _w((lambda *s: _rng.normal(s) * 0.1)(B, S, D)), 'w_r': _w((lambda *s: _rng.normal(s) * 0.1)(D)), 'w_gate': _w((lambda *s: _rng.normal(s) * 0.1)(D, F)), 'w_up': _w((lambda *s: _rng.normal(s) * 0.1)(D, F)), 'w_down': _w((lambda *s: _rng.normal(s) * 0.1)(F, D))}
    _B_in = _B_setup()
    return {'A_x': _A_in['x'], 'A_c_kv': _A_in['c_kv'], 'A_w_q': _A_in['w_q'], 'A_w_uk': _A_in['w_uk'], 'A_w_uv': _A_in['w_uv'], 'A_w_o': _A_in['w_o'], 'B_x': _B_in['x'], 'B_w_r': _B_in['w_r'], 'B_w_gate': _B_in['w_gate'], 'B_w_up': _B_in['w_up'], 'B_w_down': _B_in['w_down'], 'c': _w((lambda *s: _rng.normal(s) * 0.1)(1, 640) * 8.0), 'w_mod': _w((lambda *s: _rng.normal(s) * 0.1)(640, 6 * 640) * 640 ** (-0.5) * 8.0)}

def reference(A_x, A_c_kv, A_w_q, A_w_uk, A_w_uv, A_w_o, B_x, B_w_r, B_w_gate, B_w_up, B_w_down, c, w_mod):

    def _A_ref(x, c_kv, w_q, w_uk, w_uv, w_o):
        B, Sq, M = (x.shape[0], x.shape[1], x.shape[2])
        Sk = c_kv.shape[1]
        H, D = (w_q.shape[1], w_q.shape[2])
        q = jnp.einsum('bqm,mhd->bhqd', x, w_q)
        k = jnp.einsum('bkc,chd->bhkd', c_kv, w_uk)
        v = jnp.einsum('bkc,chd->bhkd', c_kv, w_uv)
        scores = jnp.einsum('bhqd,bhkd->bhqk', q, k) * D ** (-0.5)
        off = Sk - Sq
        qi = jnp.arange(Sq)[:, None]
        kj = jnp.arange(Sk)[None, :]
        cmask = kj <= qi + off
        scores = jnp.where(cmask[None, None], scores, -1000000000.0)
        p = _softmax(scores, axis=-1)
        ctx = jnp.einsum('bhqk,bhkd->bhqd', p, v)
        return jnp.einsum('bhqd,hdm->bqm', ctx, w_o)

    def _B_ref(x, w_r, w_gate, w_up, w_down):
        B, S, D = x.shape
        C = 8
        r = x @ w_r
        idx = jnp.argsort(-r, axis=-1)[:, :C]
        idx_e = jnp.repeat(idx.reshape(B, C, 1), D, axis=2)
        x_sel = jnp.take_along_axis(x, idx_e, axis=1)
        g = _silu(x_sel @ w_gate)
        u = x_sel @ w_up
        y = g * u @ w_down
        r_sel = _sigmoid(jnp.take_along_axis(r, idx, axis=1))
        y = y * r_sel.reshape(B, C, 1)
        b_off = (jnp.arange(B) * S).reshape(B, 1)
        flat_idx = (idx + b_off).reshape(B * C)
        zero = (x * 0.0).reshape(B * S, D)
        upd = _scatter_add(zero, flat_idx, y.reshape(B * C, D), axis=0)
        return x + upd.reshape(B, S, D)
    x = A_x
    mod = (_silu(c) @ w_mod).reshape(c.shape[0], 6, 1, -1)
    sa, ca, ga, sb, cb, gb = (mod[:, 0].copy(), mod[:, 1].copy(), mod[:, 2].copy(), mod[:, 3].copy(), mod[:, 4].copy(), mod[:, 5].copy())
    h = _layernorm(x, axis=-1) * (1 + ca) + sa
    x = x + ga * _A_ref(h, A_c_kv, A_w_q, A_w_uk, A_w_uv, A_w_o)
    h = _layernorm(x, axis=-1) * (1 + cb) + sb
    x = x + gb * _B_ref(h, B_w_r, B_w_gate, B_w_up, B_w_down)
    return x
```

```python
import jax
import jax.numpy as jnp
from jax import lax
import jax.experimental.pallas as pl
import jax.experimental.pallas.tpu as pltpu

S, M, C, H, D, F, TOPK = 2048, 640, 512, 32, 128, 1728, 8
NP = H // 2
T = 128
TQ = 256
NQ = S // TQ
PAR_N = 6
TREE_N = 4
TAIL = 40
TAIL_LAST = 40
TAIL_LN = 40
TAIL_FIN = 0
FR = 32
LR = 64
PC = 512
OB = 64
STOP = ""
UMODE = 1
CCH = [(0, 256), (256, 768), (768, 2048)]
XCH = [(1792, 2048), (1536, 1792), (768, 1536), (0, 768)]
KVSPLIT = 1664
bf = jnp.bfloat16
f32 = jnp.float32
u32 = jnp.uint32
i32 = jnp.int32
NT = (((1,), (1,)), ((), ()))
EPS = 1e-5
QSCALE = D ** -0.5 * 1.4426950408889634
NEG = -1e30
KOFF = 0x10000000


def _rb(x):
    return x.astype(bf).astype(f32)


def _dot(a, b):
    return jnp.dot(a, b, preferred_element_type=f32)


def _bits(x, dt):
    return lax.bitcast_convert_type(x, dt)


def _recip(x):
    r = pl.reciprocal(x, approx=True)
    return r * (2.0 - x * r)


def _zero_after(v):
    return jnp.where(v < 0.0, 1.0, 0.0)


def _pk2(a, b):
    return pltpu.pack_elementwise([a, b], packed_dtype=bf)


def _pack_rows(y):
    r, n = y.shape
    y4 = y.reshape(r // 16, 2, 8, n)
    return _pk2(y4[:, 0], y4[:, 1]).reshape(r // 2, n)


def _interleave(a, b):
    hi = _pk2(a, b)
    ra = a - _bits(hi << 16, f32)
    rb = b - _bits(hi & jnp.uint32(0xFFFF0000), f32)
    return pltpu.bitcast(hi, bf).astype(f32) + pltpu.bitcast(_pk2(ra, rb), bf).astype(f32)


def _asbf(u):
    return pltpu.bitcast(u, bf)


def _ln_center(x, tok=None):
    m = jnp.sum(x, axis=1, keepdims=True) * (1.0 / M)
    if tok is not None:
        m = m + tok
    xc = x - m
    v = jnp.sum(xc * xc, axis=1, keepdims=True) * (1.0 / M)
    a = _rb(_rb(v) + EPS)
    d = _rb(a * lax.rsqrt(a))
    return xc, _recip(d)


def _lo(w):
    return _bits(w << 16, f32)


def _hi(w):
    return _bits(w & jnp.uint32(0xFFFF0000), f32)


def _unpack_pair(w):
    return jnp.concatenate([_lo(w), _hi(w)], axis=1).astype(bf)


def kernel(x_hbm, c_hbm, wq_hbm, wk_hbm, wv_hbm, wo_hbm, wr_hbm, wg_hbm, wu_hbm, wd_hbm, cv_hbm, wm_hbm,
           out_hbm,
           x_s, c_s, cp_s, h_s, rq_s, rk_s, rv_s, q_s, k_s, v_s, m_s, ctx_s,
           wo_s, wr_s, wg_s, wu_s, wd_s, cv_s, wm_s, mod_s, att_s, h2_s, ob_s, out_s, key_s, tk_s,
           sem_w, sem_c, sem_x, sem_m, sem_o, sem_r, sem_b, *s_s):
    wq_u = wq_hbm.bitcast(u32)
    wk_u = wk_hbm.bitcast(u32)
    wv_u = wv_hbm.bitcast(u32)

    def w_copies(pair, slot):
        return [pltpu.make_async_copy(wk_u.at[:, pair, :], rk_s.at[slot], sem_w.at[slot, 0]),
                pltpu.make_async_copy(wv_u.at[:, pair, :], rv_s.at[slot], sem_w.at[slot, 1]),
                pltpu.make_async_copy(wq_u.at[:, pair, :], rq_s.at[slot], sem_w.at[slot, 2])]

    c_cp = [pltpu.make_async_copy(c_hbm.at[pl.ds(a, b - a)], c_s.at[pl.ds(a, b - a)], sem_c.at[i])
            for i, (a, b) in enumerate(CCH)]
    x_cp = [pltpu.make_async_copy(x_hbm.at[pl.ds(a, b - a)], x_s.at[pl.ds(a, b - a)], sem_x.at[i])
            for i, (a, b) in enumerate(XCH)]
    cv_cp = pltpu.make_async_copy(cv_hbm, cv_s, sem_m.at[0])
    wm0_cp = pltpu.make_async_copy(wm_hbm.at[:, pl.ds(0, 2 * M)], wm_s.at[:, pl.ds(0, 2 * M)], sem_m.at[1])
    late_cp = [pltpu.make_async_copy(wm_hbm.at[:, pl.ds(2 * M, 4 * M)], wm_s.at[:, pl.ds(2 * M, 4 * M)], sem_m.at[2]),
               pltpu.make_async_copy(wo_hbm, wo_s, sem_m.at[3]),
               pltpu.make_async_copy(wr_hbm, wr_s, sem_m.at[4]),
               pltpu.make_async_copy(wg_hbm, wg_s, sem_m.at[5]),
               pltpu.make_async_copy(wu_hbm, wu_s, sem_m.at[6]),
               pltpu.make_async_copy(wd_hbm, wd_s, sem_m.at[7])]

    def stop():
        fin = pltpu.make_async_copy(out_s.at[pl.ds(0, 16)], out_hbm.at[pl.ds(0, 16)], sem_o.at[0])
        fin.start(); fin.wait()

    def bar():
        pl.semaphore_signal(sem_b, 1)
        pl.semaphore_wait(sem_b, 1)

    def urgent(z, n):
        for _ in range(n):
            if UMODE == 0:
                tk_s[:, 0:T] = jnp.concatenate([z, z], axis=0).astype(bf)
                z = tk_s[:, 0:T].astype(f32)[0:8]
            elif UMODE == 1:
                tk_s[0:8, 0:T] = z.astype(bf)
                z = tk_s[0:8, 0:T].astype(f32)
        return z

    def rows(ref, a, b):
        return _asbf(ref[a // 2:b // 2, :])

    def rows3(ref, e, a, b):
        return _asbf(ref[e, a // 2:b // 2, :])

    def proj(lhs, w, dst, a, b):
        y = _pack_rows(_dot(lhs, w))
        dst[0, a // 2:b // 2, :] = y[:, 0:D]
        dst[1, a // 2:b // 2, :] = y[:, D:2 * D]

    row = lax.broadcasted_iota(i32, (T, T), 0)
    col = lax.broadcasted_iota(i32, (T, T), 1)
    row = (row & ~15) | ((row & 15) >> 2) | ((row & 3) << 2)
    col = (col & ~15) | ((col & 15) >> 1) | ((col & 1) << 3)
    mask = col <= row

    def qk(e, i):
        r0 = i * TQ
        s = lax.dot_general(rows3(q_s, e, r0, r0 + TQ), rows3(k_s, e, 0, r0 + T), NT, preferred_element_type=f32)
        s2 = lax.dot_general(rows3(q_s, e, r0 + T, r0 + TQ), rows3(k_s, e, r0 + T, r0 + TQ), NT,
                             preferred_element_type=f32)
        dtop = jnp.where(mask, s[0:T, r0:r0 + T], NEG)
        top = jnp.concatenate([s[0:T, 0:r0], dtop], axis=1) if r0 > 0 else dtop
        bot = jnp.concatenate([s[T:TQ, :], jnp.where(mask, s2, NEG)], axis=1)
        s_s[e * NQ + i][0:T, 0:r0 + T] = top
        s_s[e * NQ + i][T:TQ, :] = bot
        m_s[e, r0:r0 + T, :] = jnp.broadcast_to(jnp.max(top, axis=1, keepdims=True), (T, D))
        m_s[e, r0 + T:r0 + TQ, :] = jnp.broadcast_to(jnp.max(bot, axis=1, keepdims=True), (T, D))

    def pv(e, i, pair, P):
        r0 = i * TQ
        ptop = jnp.concatenate([u[0] for u in P[0:T // 16]], axis=0)
        pbot = jnp.concatenate([u[0] for u in P[T // 16:]], axis=0)
        rl = jnp.concatenate([u[1] for u in P], axis=0)
        ctx = _dot(_asbf(jnp.concatenate([ptop, pbot[:, 0:r0 + T]], axis=0)), rows3(v_s, e, 0, r0 + T))
        c2 = _dot(_asbf(pbot[:, r0 + T:r0 + TQ]), rows3(v_s, e, r0 + T, r0 + TQ))
        ctx = jnp.concatenate([ctx[0:T], ctx[T:TQ] + c2], axis=0)
        ctx_s[2 * pair + e, r0 // 2:(r0 + TQ) // 2, :] = _pack_rows(ctx * rl)

    order = list(range(NQ))[::-1]

    def scores(e):
        for i in order:
            qk(e, i)

    def fold(x, n, op):
        parts = [x[:, t * T:(t + 1) * T] for t in range(n)]
        nacc = 2 if n >= TREE_N else 1
        accs = parts[:nacc]
        for t in range(nacc, n):
            accs[t % nacc] = op(accs[t % nacc], parts[t])
        return accs[0] if nacc == 1 else op(accs[0], accs[1])

    def softmax(tok):
        P = {}
        for e in range(2):
            for i in order:
                P[(e, i)] = []
                for rr in range(0, TQ, 16):
                    n = (i * TQ + rr) // T + 1
                    L = n * T
                    ps, accs, ls = [], [], []
                    for half in range(2):
                        r8 = rr + 8 * half
                        r = i * TQ + r8
                        me = m_s[e, r:r + 8, :] + tok
                        p = jnp.exp2(s_s[e * NQ + i][r8:r8 + 8, 0:L] - jnp.concatenate([me] * n, axis=1))
                        acc = fold(p, n, jnp.add)
                        ls.append(jnp.broadcast_to(jnp.sum(acc, axis=1, keepdims=True), (8, D)))
                        ps.append(p)
                        accs.append(acc)
                        if half == 0 and n > PAR_N:
                            tok = _zero_after(acc)
                    pk = _pk2(ps[0], ps[1])
                    z = fold(pk, n, jnp.bitwise_or) | _bits(accs[1], u32)
                    if n <= PAR_N:
                        z = z | _bits(accs[0], u32)
                    tok = jnp.where(_bits(z, i32) < 0, 1.0, 0.0)
                    P[(e, i)].append((pk, _recip(_interleave(ls[0], ls[1]))))
        return P, tok

    def values(e, pair, P):
        for i in order:
            pv(e, i, pair, P[(e, i)])

    def silu_c():
        cvec = cv_s[...].astype(f32)
        return jnp.broadcast_to((cvec * jax.nn.sigmoid(cvec)).astype(bf), (8, M))

    w0 = w_copies(0, 0)
    for cp in [w0[0], c_cp[0], w0[1], c_cp[1], c_cp[2], cv_cp, wm0_cp, x_cp[0], w0[2]] + x_cp[1:]:
        cp.start()
        bar()
    for cp in w_copies(1, 1): cp.start()
    bar()
    for cp in late_cp: cp.start(priority=1)

    def kv(a, b, wk, wv):
        lhs = c_s[a:b, :]
        cp_s[a // 2:b // 2, :] = pltpu.bitcast(lhs, u32)
        proj(lhs, wk, k_s, a, b)
        proj(lhs, wv, v_s, a, b)

    def ln1(i, ztok):
        tok = None
        z = None
        for a in range(XCH[i][1] - LR, XCH[i][0] - 1, -LR):
            xc, rinv = _ln_center(x_s[a:a + LR, :].astype(f32), tok)
            tok = _zero_after(rinv)
            hp = _pack_rows(xc * rinv * mod_s[0:1, 0:M] + mod_s[0:1, M:2 * M])
            h_s[a // 2:(a + LR) // 2, :] = hp
        return urgent(ztok + jnp.broadcast_to(tok[0:8], (8, T)), TAIL_LN)

    def qblock(i, wq):
        proj(rows(h_s, i * TQ, (i + 1) * TQ), wq, q_s, i * TQ, (i + 1) * TQ)
        qk(0, i)
        qk(1, i)

    tok = jnp.zeros((8, T), f32)
    w0[0].wait(); c_cp[0].wait(); w0[1].wait()
    wk = _unpack_pair(rk_s[0])
    wv = _unpack_pair(rv_s[0])
    kv(*CCH[0], wk, wv)
    c_cp[1].wait()
    kv(*CCH[1], wk, wv)
    c_cp[2].wait()
    kv(CCH[2][0], KVSPLIT, wk, wv)
    cv_cp.wait(); wm0_cp.wait(); x_cp[0].wait()
    mod0 = _rb(_dot(silu_c(), wm_s[:, 0:2 * M]))
    mod_s[:, 0:M] = _rb(1.0 + mod0[:, M:2 * M]) * QSCALE
    mod_s[:, M:2 * M] = mod0[:, 0:M] * QSCALE
    kv(KVSPLIT, S, wk, wv)
    tok = ln1(0, tok)
    w0[2].wait(); x_cp[1].wait()
    wq = _unpack_pair(rq_s[0])
    qblock(7, wq)
    tok = ln1(1, tok)
    x_cp[2].wait()
    qblock(6, wq)
    tok = ln1(2, tok)
    x_cp[3].wait()
    tok = ln1(3, tok)
    for i in range(5, -1, -1):
        qblock(i, wq)

    if STOP == "P":
        pl.delay(40000)
        for cp in w_copies(1, 1) + late_cp: cp.wait()
        acc = tok
        for r in s_s: acc = acc + r[0:8, 0:T] + r[TQ - 8:TQ, 0:T]
        out_s[0:8, 0:128] = (acc + m_s[0, 0:8] + _bits(v_s[0, 0:8], f32) + _bits(cp_s[0:8, 0:T], f32)).astype(bf)
        return stop()
    def body(j, tok):
        nslot = (j + 1) & 1
        for cp in w_copies(j + 1, nslot): cp.wait()
        P, tok = softmax(tok)
        wq = _unpack_pair(rq_s[nslot])

        @pl.when(j + 2 < NP)
        def _():
            for cp in w_copies(j + 2, j & 1): cp.start()

        for a in range(0, S, PC): proj(rows(h_s, a, a + PC), wq, q_s, a, a + PC)
        wk = _unpack_pair(rk_s[nslot])
        for a in range(0, S, PC): proj(rows(cp_s, a, a + PC), wk, k_s, a, a + PC)

        def vproj(e):
            wv = (_lo, _hi)[e](rv_s[nslot]).astype(bf)
            for a in range(0, S, PC):
                v_s[e, a // 2:(a + PC) // 2, :] = _pack_rows(_dot(rows(cp_s, a, a + PC), wv))

        values(0, j, P)
        vproj(0)
        values(1, j, P)
        scores(0)
        scores(1)
        vproj(1)
        return urgent(tok, TAIL)

    tok = lax.fori_loop(0, NP - 1, body, tok)

    for cp in late_cp: cp.wait()
    if STOP == "L1":
        out_s[0:16, 0:128] = _asbf(ctx_s[3, 0:8, :] + ctx_s[5, 16:24, :])
        return stop()

    def oproj(r0, h0, h1):
        lhs = jnp.concatenate([ctx_s[h, pl.ds(r0 // 2, TQ // 2), :] for h in range(h0, h1)], axis=1)
        return _dot(_asbf(lhs), wo_s[h0 * D:h1 * D, :])

    P, tok = softmax(tok)
    att_s[...] = oproj((NQ - 1) * TQ, 0, H - 2)
    mod_s[...] = _rb(_dot(silu_c(), wm_s[:, 2 * M:6 * M]))
    values(0, NP - 1, P)
    values(1, NP - 1, P)
    att_s[...] += oproj((NQ - 1) * TQ, H - 2, H)
    key0 = urgent(tok, TAIL_LAST)
    key_s[0] = key0
    key_s[1] = key0

    def out_copy(blk):
        r0 = pl.multiple_of(blk * TQ, TQ)
        return pltpu.make_async_copy(out_s.at[pl.ds(r0, TQ)], out_hbm.at[pl.ds(r0, TQ)], sem_o.at[blk])

    def finish(blk, throttle):
        r0 = pl.multiple_of(blk * TQ, TQ)
        ga = mod_s[0:1, 0:M]
        sb = mod_s[0:1, M:2 * M]
        cb1 = _rb(1.0 + mod_s[0:1, 2 * M:3 * M])
        gb = mod_s[0:1, 3 * M:4 * M]
        wr = wr_s[...].astype(f32).reshape(1, M)
        tok = None
        kmax = None
        for a in range(0, TQ, FR):
            ra = pl.multiple_of(r0 + a, FR)
            x1 = x_s[pl.ds(ra, FR), :].astype(f32) + ga * att_s[a:a + FR, :]
            xc, rinv = _ln_center(x1, tok)
            h2 = xc * rinv * cb1 + sb
            h2_s[pl.ds(ra, FR), :] = h2
            ob = x1 + gb * h2
            ob_s[pl.ds(ra, FR), :] = ob
            out_s[pl.ds(ra, FR), :] = ob.astype(bf)
            r = _rb(jnp.sum(h2 * wr, axis=1, keepdims=True)) + 0.0
            if throttle:
                tok = _zero_after(r * r)
            b = _bits(jnp.broadcast_to(r, (FR, T)), i32) >> 16
            o = jnp.where(b < 0, ~b, b + 32768 - 0) if False else jnp.where(b < 0, -1 - b, b + 32768)
            o = jnp.where(b < 0, 32767 - (b & 32767), b + 32768)
            rws = lax.broadcasted_iota(i32, (FR, T), 0) + ra
            lane = lax.broadcasted_iota(i32, (FR, T), 1)
            key = _bits((o << 11) + (KOFF + S - 1 - rws), f32)
            key = jnp.where(lane == ((rws >> 3) & (T - 1)), key, 0.0)
            key = jnp.max(key.reshape(FR // 8, 8, T), axis=0)
            kmax = key if kmax is None else jnp.maximum(kmax, key)
        hi = blk // 4
        key_s[hi] = jnp.maximum(key_s[hi], kmax)
        out_copy(blk).start()

    def body2(t, carry):
        blk = NQ - 2 - t
        finish(blk + 1, True)
        att_s[...] = oproj(pl.multiple_of(blk * TQ, TQ), 0, H)
        return carry

    lax.fori_loop(0, NQ - 1, body2, 0)
    if STOP == "L2":
        for blk in range(1, NQ): out_copy(blk).wait()
        out_s[0:16, :] = att_s[0:16, :].astype(bf)
        return stop()
    finish(0, False)

    keys = key_s[...].reshape(16, T)
    sub = lax.broadcasted_iota(i32, (TOPK, T), 0)
    sel = jnp.zeros((TOPK, T), f32)
    idxs = []
    for k in range(TOPK):
        mx = jnp.max(jnp.max(keys, axis=0, keepdims=True), axis=1, keepdims=True)
        keys = jnp.where(keys == mx, 0.0, keys)
        sel = jnp.where(sub == k, mx, sel)
        idxs.append(jnp.clip(S - 1 - (_bits(mx, i32)[0, 0] & (S - 1)), 0, S - 1))
    xs = jnp.concatenate([h2_s[pl.ds(ix, 1), :] for ix in idxs], axis=0).astype(bf)
    g = _rb(lax.dot_general(xs, wg_s[...], NT, preferred_element_type=f32))
    g = _rb(g * jax.nn.sigmoid(g))
    u = _rb(lax.dot_general(xs, wu_s[...], NT, preferred_element_type=f32))
    y = _rb(_dot((g * u).astype(bf), wd_s[...]))
    o = ((_bits(sel, i32) - KOFF) >> 11) & 65535
    rsel = _bits(jnp.where(o >= 32768, o - 32768, 65535 - o) << 16, f32)
    sig = _rb(jax.nn.sigmoid(rsel))[:, 0:1]
    upd = mod_s[0:1, 3 * M:4 * M] * (y * sig)
    for k in range(TOPK):
        ob_s[pl.ds(idxs[k], 1), :] = ob_s[pl.ds(idxs[k], 1), :] + upd[k:k + 1, :]
    for blk in range(NQ):
        out_copy(blk).wait()
    for k in range(TOPK):
        g0 = pl.multiple_of((idxs[k] >> 4) << 4, 16)
        out_s[pl.ds(g0, 16), :] = ob_s[pl.ds(g0, 16), :].astype(bf)
    hit = 0
    for k in range(TOPK):
        hit = hit | (jnp.int32(1) << (idxs[k] // OB))
    resend = [pltpu.make_async_copy(out_s.at[pl.ds(b * OB, OB)], out_hbm.at[pl.ds(b * OB, OB)], sem_r.at[b])
              for b in range(S // OB)]
    for b in range(S // OB):
        pl.when(((hit >> b) & 1) == 1)(resend[b].start)
    for b in range(S // OB):
        pl.when(((hit >> b) & 1) == 1)(resend[b].wait)


@jax.jit
def pallas_adaLN_cond__compressed_kv_cla__moe_arch_mod__prompt_kernel(A_x, A_c_kv, A_w_q, A_w_uk, A_w_uv, A_w_o, B_x, B_w_r, B_w_gate, B_w_up, B_w_down, c, w_mod):
    V = pltpu.VMEM
    scratch = [
        V((S, M), bf), V((S, C), bf), V((S // 2, C), u32), V((S // 2, M), u32),
        V((2, M, D), u32), V((2, C, D), u32), V((2, C, D), u32),
        V((2, S // 2, D), u32), V((2, S // 2, D), u32), V((2, S // 2, D), u32),
        V((2, S, D), f32), V((H, S // 2, D), u32),
        V((H * D, M), bf), V((M,), bf), V((F, M), bf), V((F, M), bf), V((F, M), bf),
        V((1, M), bf), V((M, 6 * M), bf), V((8, 4 * M), f32),
        V((TQ, M), f32), V((S, M), f32), V((S, M), f32), V((S, M), bf), V((2, 8, T), f32), V((16, 2 * T), bf),
        pltpu.SemaphoreType.DMA((2, 3)), pltpu.SemaphoreType.DMA((len(CCH),)), pltpu.SemaphoreType.DMA((len(XCH),)),
        pltpu.SemaphoreType.DMA((8,)), pltpu.SemaphoreType.DMA((NQ,)), pltpu.SemaphoreType.DMA((S // OB,)),
        pltpu.SemaphoreType.REGULAR,
    ] + [V((TQ, (i + 1) * TQ), f32) for _ in range(2) for i in range(NQ)]
    out = pl.pallas_call(
        kernel,
        in_specs=[pl.BlockSpec(memory_space=pltpu.HBM)] * 12,
        out_specs=pl.BlockSpec(memory_space=pltpu.HBM),
        out_shape=jax.ShapeDtypeStruct((S, M), bf),
        scratch_shapes=scratch,
        compiler_params=pltpu.CompilerParams(vmem_limit_bytes=120 * 1024 * 1024, disable_bounds_checks=True),
    )(A_x.reshape(S, M), A_c_kv.reshape(S, C), A_w_q, A_w_uk, A_w_uv, A_w_o.reshape(H * D, M),
      B_w_r, B_w_gate.T, B_w_up.T, B_w_down, c, w_mod)
    return out.reshape(1, S, M)
```

```python
import jax
import jax.numpy as jnp
from jax import lax
import jax.experimental.pallas as pl
import jax.experimental.pallas.tpu as pltpu

S, M, C, H, D, F, TOPK = 2048, 640, 512, 32, 128, 1728, 8
NP = H // 2
T = 128
TQ = 256
NQ = S // TQ
FP = 1792
PC = 512
FR = 16
GR = 8
PAR_N = 6
LK = 8
NURG = 32
CCH = [(0, 256), (256, 768), (768, 2048)]
XCH = [(1792, 2048), (1536, 1792), (0, 1536)]
K1 = 896
K2 = 1664
K3 = 1792
bf = jnp.bfloat16
f32 = jnp.float32
u32 = jnp.uint32
i32 = jnp.int32
NT = (((1,), (1,)), ((), ()))
EPS = 1e-5
QSCALE = D ** -0.5 * 1.4426950408889634
NEG = -1e30
KOFF = 0x10000000
KHALF = 1 << 18


def _rb(x):
    return x.astype(bf).astype(f32)


def _dot(a, b):
    return jnp.dot(a, b, preferred_element_type=f32)


def _bits(x, dt):
    return lax.bitcast_convert_type(x, dt)


def _recip(x):
    r = pl.reciprocal(x, approx=True)
    return r * (2.0 - x * r)


def _zero_after(v):
    return jnp.where(v < 0.0, 1.0, 0.0)


def _rowwise(x, w8, op):
    r, n = x.shape
    return op(x.reshape(r // 8, 8, n), w8[None]).reshape(r, n)


def _fold(x):
    n = x.shape[1] // T
    parts = [x[:, t * T:(t + 1) * T] for t in range(n)]
    nacc = 2 if n >= 4 else 1
    accs = parts[:nacc]
    for t in range(nacc, n):
        accs[t % nacc] = accs[t % nacc] + parts[t]
    return accs[0] if nacc == 1 else accs[0] + accs[1]


def _tile_lanes(v, n):
    return jnp.concatenate([v] * n, axis=1)


def _unpack_pair(w):
    lo = _bits(w << 16, f32)
    hi = _bits(w & jnp.uint32(0xFFFF0000), f32)
    return jnp.concatenate([lo, hi], axis=1).astype(bf)


def _top8(keys):
    keys = keys.reshape(keys.shape[0] // 8, 8, T)
    sub = lax.broadcasted_iota(i32, (8, T), 0)
    top = jnp.zeros((8, T), f32)
    for k in range(TOPK):
        mx = jnp.max(jnp.max(keys, axis=0), axis=0, keepdims=True)
        top = jnp.where(sub == k, mx, top)
        if k + 1 < TOPK:
            keys = jnp.where(keys == mx[None], 0.0, keys)
    return top


def _kernel(x_hbm, c_hbm, wq_hbm, wk_hbm, wv_hbm, wo_hbm, wr_hbm, wg_hbm, wu_hbm, wd_hbm, cv_hbm, wm_hbm,
            out_hbm,
            x_s, c_s, cp_s, h_s, rq_s, rk_s, rv_s, q_s, k0_s, k_s, v_s, m_s, ctx_s,
            wo_s, wr_s, wg_s, wu_s, wd_s, wt_s, cv_s, sc_s, wm_s, mod_s, att_s, h2_s, ob_s, out_s,
            key_s, fix_s, tk_s,
            sem_w, sem_c, sem_x, sem_m, sem_o, sem_b, *s_s):
    def w_copy(w_hbm, dst, sem_col, pair, slot):
        return pltpu.make_async_copy(w_hbm.bitcast(u32).at[:, pair, :], dst.at[slot], sem_w.at[slot, sem_col])

    def step_copies(j, par):
        return [w_copy(wq_hbm, rq_s, 2, j + 1, 1 - par), w_copy(wv_hbm, rv_s, 1, j + 1, 1 - par),
                w_copy(wk_hbm, rk_s, 0, jnp.minimum(j + 2, NP - 1), par)]

    c_cp = [pltpu.make_async_copy(c_hbm.at[pl.ds(a, b - a)], c_s.at[pl.ds(a, b - a)], sem_c.at[i])
            for i, (a, b) in enumerate(CCH)]
    x_cp = [pltpu.make_async_copy(x_hbm.at[pl.ds(a, b - a)], x_s.at[pl.ds(a, b - a)], sem_x.at[i])
            for i, (a, b) in enumerate(XCH)]
    cv_cp = pltpu.make_async_copy(cv_hbm, cv_s, sem_m.at[0])
    wm0_cp = pltpu.make_async_copy(wm_hbm.at[:, pl.ds(0, 2 * M)], wm_s.at[:, pl.ds(0, 2 * M)], sem_m.at[1])
    late_cp = [pltpu.make_async_copy(wm_hbm.at[:, pl.ds(2 * M, 4 * M)], wm_s.at[:, pl.ds(2 * M, 4 * M)], sem_m.at[2]),
               pltpu.make_async_copy(wo_hbm, wo_s, sem_m.at[3]),
               pltpu.make_async_copy(wr_hbm, wr_s, sem_m.at[4]),
               pltpu.make_async_copy(wg_hbm, wg_s.at[pl.ds(0, F)], sem_m.at[5]),
               pltpu.make_async_copy(wu_hbm, wu_s.at[pl.ds(0, F)], sem_m.at[6]),
               pltpu.make_async_copy(wd_hbm, wd_s.at[pl.ds(0, F)], sem_m.at[7])]

    def out_copy(blk):
        r0 = pl.multiple_of(blk * TQ, TQ)
        return pltpu.make_async_copy(out_s.at[pl.ds(r0, TQ)], out_hbm.at[pl.ds(r0, TQ)], sem_o.at[blk])

    def fence():
        pl.semaphore_signal(sem_b, 1)
        pl.semaphore_wait(sem_b, 1)

    def urgent(z, par=None):
        src = 0 if par is None else 1 - par
        dst = 0 if par is None else par
        for _ in range(NURG):
            tk_s[dst, 0:8, 0:T] = z.astype(bf)
            z = tk_s[src, 0:8, 0:T].astype(f32)
        return z

    def proj(lhs, w, dst, a, b):
        y = _dot(lhs, w)
        dst[0, a:b, :] = y[:, 0:D].astype(bf)
        dst[1, a:b, :] = y[:, D:2 * D].astype(bf)

    def c_rows(a, b):
        return pltpu.bitcast(cp_s[a // 2:b // 2, :], bf)

    causal = lax.broadcasted_iota(i32, (T, T), 1) <= lax.broadcasted_iota(i32, (T, T), 0)
    order = list(range(NQ))[::-1]

    def qk(e, i, kref):
        r0 = i * TQ
        s = lax.dot_general(q_s[e, r0:r0 + TQ, :], kref[e, 0:r0 + T, :], NT, preferred_element_type=f32)
        s2 = lax.dot_general(q_s[e, r0 + T:r0 + TQ, :], kref[e, r0 + T:r0 + TQ, :], NT, preferred_element_type=f32)
        dtop = jnp.where(causal, s[0:T, r0:r0 + T], NEG)
        top = jnp.concatenate([s[0:T, 0:r0], dtop], axis=1) if r0 > 0 else dtop
        bot = jnp.concatenate([s[T:TQ, :], jnp.where(causal, s2, NEG)], axis=1)
        s_s[e * NQ + i][0:T, 0:r0 + T] = top
        s_s[e * NQ + i][T:TQ, :] = bot
        m_s[e, r0:r0 + T, :] = jnp.broadcast_to(jnp.max(top, axis=1, keepdims=True), (T, D))
        m_s[e, r0 + T:r0 + TQ, :] = jnp.broadcast_to(jnp.max(bot, axis=1, keepdims=True), (T, D))

    def softmax(tok):
        P = {}
        for e in range(2):
            for i in order:
                P[(e, i)] = []
                prev = None
                for rr in range(0, TQ, 8):
                    r = i * TQ + rr
                    n = r // T + 1
                    m = m_s[e, r:r + 8, :] + tok
                    p = jnp.exp2(s_s[e * NQ + i][rr:rr + 8, 0:n * T] - _tile_lanes(m, n))
                    acc = _fold(p)
                    P[(e, i)].append((p, acc))
                    if n > PAR_N:
                        tok = _zero_after(acc)
                    elif prev is None:
                        prev = acc
                    else:
                        tok = _zero_after(acc + prev)
                        prev = None
        return P, tok

    def values(e, pair, P):
        for i in order:
            r0 = i * TQ
            units = P[(e, i)]
            ptop = jnp.concatenate([u[0] for u in units[0:T // 8]], axis=0)
            pbot = jnp.concatenate([u[0] for u in units[T // 8:]], axis=0)
            l = jnp.sum(jnp.concatenate([u[1] for u in units], axis=0), axis=1, keepdims=True)
            ctx = _dot(jnp.concatenate([ptop, pbot[:, 0:r0 + T]], axis=0).astype(bf), v_s[e, 0:r0 + T, :])
            c2 = _dot(pbot[:, r0 + T:r0 + TQ].astype(bf), v_s[e, r0 + T:r0 + TQ, :])
            ctx = jnp.concatenate([ctx[0:T], ctx[T:TQ] + c2], axis=0)
            ctx_s[2 * pair + e, r0:r0 + TQ, :] = (ctx * _recip(l)).astype(bf)

    def ln1(i, tok):
        starts = list(range(XCH[i][1] - 8, XCH[i][0] - 1, -8))
        nu = len(starts)
        mean, rinv = {}, {}
        for t in range(nu + 2 * LK):
            if t < nu:
                a = starts[t]
                s1 = _fold(x_s[a:a + 8, :].astype(f32)) + tok
                mean[t] = jnp.sum(s1, axis=1, keepdims=True) * (1.0 / M)
                tok = _zero_after(s1 * s1)
            u = t - LK
            if 0 <= u < nu:
                a = starts[u]
                xc = x_s[a:a + 8, :].astype(f32) - _tile_lanes(mean[u] + tok, M // T)
                s2 = _fold(xc * xc)
                rinv[u] = lax.rsqrt(jnp.sum(s2, axis=1, keepdims=True) * (1.0 / M) + EPS)
                tok = _zero_after(s2)
            u = t - 2 * LK
            if 0 <= u < nu:
                a = starts[u]
                xn = (x_s[a:a + 8, :].astype(f32) - mean[u]) * _tile_lanes(rinv[u] + tok, M // T)
                hv = xn * mod_s[:, 0:M] + mod_s[:, M:2 * M]
                h_s[a:a + 8, :] = hv.astype(bf)
                z = _fold(hv)
                tok = _zero_after(z * z)
        return urgent(tok)

    wk0_cp, wv0_cp, wq0_cp = w_copy(wk_hbm, rk_s, 0, 0, 0), w_copy(wv_hbm, rv_s, 1, 0, 0), w_copy(wq_hbm, rq_s, 2, 0, 0)
    wk1_cp = w_copy(wk_hbm, rk_s, 0, 1, 1)
    for cp in [cv_cp, wk0_cp, c_cp[0], wv0_cp, c_cp[1], wk1_cp, c_cp[2], wm0_cp, x_cp[0], wq0_cp] + x_cp[1:]:
        cp.start()
        fence()

    tok = jnp.zeros((8, T), f32)
    for w_ in (wg_s, wu_s, wd_s):
        w_[F:FP, :] = jnp.zeros((FP - F, M), bf)
    tk_s[...] = jnp.zeros(tk_s.shape, bf)
    cv_cp.wait()
    cvec = cv_s[...].astype(f32)
    silu_c = _rb(cvec * jax.nn.sigmoid(cvec))
    sc_s[...] = jnp.broadcast_to(silu_c, (T, M)).T
    wk0_cp.wait(); c_cp[0].wait(); wv0_cp.wait()
    wk0 = _unpack_pair(rk_s[0])
    wv0 = _unpack_pair(rv_s[0])

    def kv0(a, b):
        lhs = c_s[a:b, :]
        cp_s[a // 2:b // 2, :] = pltpu.bitcast(lhs, u32)
        proj(lhs, wk0, k0_s, a, b)
        proj(lhs, wv0, v_s, a, b)

    kv0(*CCH[0])
    c_cp[1].wait()
    kv0(*CCH[1])
    wk1_cp.wait()
    wk1 = _unpack_pair(rk_s[1])

    def k1(a, b):
        proj(c_s[a:b, :], wk1, k_s, a, b)

    k1(0, CCH[2][0])
    c_cp[2].wait()
    kv0(*CCH[2])
    k1(CCH[2][0], K1)
    wm0_cp.wait(); x_cp[0].wait()
    mod0 = _rb(_dot(jnp.broadcast_to(silu_c.astype(bf), (8, M)), wm_s[:, 0:2 * M]))
    mod_s[:, 0:M] = _rb(1.0 + mod0[:, M:2 * M]) * QSCALE
    mod_s[:, M:2 * M] = mod0[:, 0:M] * QSCALE
    k1(K1, K2)
    tok = ln1(0, tok)
    wq0_cp.wait(); x_cp[1].wait()
    wq0 = _unpack_pair(rq_s[0])

    def q0(i):
        proj(h_s[i * TQ:(i + 1) * TQ, :], wq0, q_s, i * TQ, (i + 1) * TQ)

    tok = ln1(1, tok)
    q0(7)
    qk(0, 7, k0_s); qk(1, 7, k0_s)
    q0(6)
    for cp in step_copies(0, 0):
        cp.start()
    for cp in late_cp:
        cp.start(priority=1)
    x_cp[2].wait()
    tok = ln1(2, tok)
    qk(0, 6, k0_s); qk(1, 6, k0_s)
    q0(5)
    k1(K2, K3)
    for i in range(5, -1, -1):
        qk(0, i, k0_s)
        if i > 0:
            q0(i - 1)
        qk(1, i, k0_s)
    k1(K3, S)

    def step(j, tok, last):
        par = j & 1
        for cp in step_copies(j, par):
            cp.wait()
        P, tok = softmax(tok)
        wq = _unpack_pair(rq_s[1 - par])
        if not last:
            for cp in step_copies(j + 1, 1 - par):
                cp.start()
        for a in range(0, S, PC):
            proj(h_s[a:a + PC, :], wq, q_s, a, a + PC)

        def vproj():
            wv = _unpack_pair(rv_s[1 - par])
            for a in range(0, S, PC):
                proj(c_rows(a, a + PC), wv, v_s, a, a + PC)

        values(0, j, P)
        values(1, j, P)
        if not last:
            vproj()
        for e in range(2):
            for i in order:
                qk(e, i, k_s)
        if last:
            vproj()
        else:
            wk = _unpack_pair(rk_s[par])
            for a in range(S - PC, -1, -PC):
                proj(c_rows(a, a + PC), wk, k_s, a, a + PC)
        return urgent(tok, None if last else par)
    tok = lax.fori_loop(0, NP - 2, lambda j, t: step(j, t, False), tok)
    tok = step(NP - 2, tok, True)

    for cp in late_cp:
        cp.wait()

    def oproj(r0, h0, h1):
        lhs = jnp.concatenate([ctx_s[h, pl.ds(r0, TQ), :] for h in range(h0, h1)], axis=1)
        return _dot(lhs, wo_s[h0 * D:h1 * D, :])

    cols = []
    for jt in range(4 * M // T):
        w = wm_s[:, 2 * M + jt * T:2 * M + (jt + 1) * T].astype(f32)
        acc = None
        for g in range(M // 8):
            t_ = (w[8 * g:8 * g + 8, :] + tok) * sc_s[8 * g:8 * g + 8, :]
            acc = t_ if acc is None else acc + t_
            if (g + 1) % 16 == 0:
                tok = _zero_after(acc * acc)
        cols.append(jnp.broadcast_to(jnp.sum(acc, axis=0, keepdims=True), (8, T)))
    mod1 = _rb(jnp.concatenate(cols, axis=1))
    P, tok = softmax(tok)
    att_s[...] = oproj((NQ - 1) * TQ, 0, H - 2)
    mod_s[:, 0:2 * M] = mod1[:, 0:2 * M]
    mod_s[:, 2 * M:3 * M] = _rb(1.0 + mod1[:, 2 * M:3 * M])
    mod_s[:, 3 * M:4 * M] = mod1[:, 3 * M:4 * M]
    mod_s[:, 4 * M:5 * M] = jnp.broadcast_to(wr_s[...].astype(f32).reshape(1, M), (8, M))
    values(0, NP - 1, P)
    values(1, NP - 1, P)
    att_s[...] += oproj((NQ - 1) * TQ, H - 2, H)
    key_s[...] = urgent(tok)

    def finish(blk, paced):
        r0 = pl.multiple_of(blk * TQ, TQ)
        ga, sb, cb1, gb, wr = [mod_s[:, k * M:(k + 1) * M] for k in range(5)]
        tok = None
        keys = [key_s[...]]
        for a in range(0, TQ, FR):
            ra = pl.multiple_of(r0 + a, FR)
            x1 = x_s[pl.ds(ra, FR), :].astype(f32) + _rowwise(att_s[a:a + FR, :], ga, jnp.multiply)
            m = jnp.sum(x1, axis=1, keepdims=True) * (1.0 / M)
            if tok is not None:
                m = m + tok
            xc = x1 - m
            rinv = lax.rsqrt(jnp.sum(xc * xc, axis=1, keepdims=True) * (1.0 / M) + EPS)
            h2 = _rowwise(_rowwise(xc * rinv, cb1, jnp.multiply), sb, jnp.add)
            h2_s[pl.ds(ra, FR), :] = h2
            ob = x1 + _rowwise(h2, gb, jnp.multiply)
            ob_s[pl.ds(ra, FR), :] = ob
            out_s[pl.ds(ra, FR), :] = ob.astype(bf)
            r = jnp.sum(_rowwise(h2, wr, jnp.multiply), axis=1, keepdims=True) + 0.0
            if paced:
                tok = _zero_after(r * r)
            b = _bits(jnp.broadcast_to(r, (FR, T)), i32) >> 13
            o = jnp.where(b < 0, (KHALF - 1) - (b & (KHALF - 1)), b + KHALF)
            rws = lax.broadcasted_iota(i32, (FR, T), 0) + ra
            keys.append(_bits((o << 11) + (KOFF + S - 1 - rws), f32))
            if paced or a + FR == TQ:
                keys = [_top8(jnp.concatenate(keys, axis=0))]
        key_s[...] = keys[0]
        out_copy(blk).start()

    def oblock(t, carry):
        blk = NQ - 2 - t
        finish(blk + 1, True)
        f0 = pl.multiple_of(t * TQ, TQ)
        wt_s[0, t] = wg_s[pl.ds(f0, TQ), :].T
        wt_s[1, t] = wu_s[pl.ds(f0, TQ), :].T
        att_s[...] = oproj(pl.multiple_of(blk * TQ, TQ), 0, H)
        return carry
    lax.fori_loop(0, NQ - 1, oblock, 0)
    finish(0, False)

    sel = _bits(key_s[...], i32)
    rowid = (S - 1) - (sel & (S - 1))
    idxs = [jnp.clip(rowid[k, 0], 0, S - 1) for k in range(TOPK)]
    xs = jnp.concatenate([h2_s[pl.ds(ix, 1), :] for ix in idxs], axis=0).astype(bf)
    g = _rb(_dot(xs, jnp.concatenate([wt_s[0, t] for t in range(NQ - 1)], axis=1)))
    g = _rb(g * jax.nn.sigmoid(g))
    u = _rb(_dot(xs, jnp.concatenate([wt_s[1, t] for t in range(NQ - 1)], axis=1)))
    y = _rb(_dot((g * u).astype(bf), wd_s[...]))
    o = (sel - KOFF) >> 11
    rsel = _bits((jnp.where(o >= KHALF, o - KHALF, 2 * KHALF - 1 - o) << 13) | 4096, f32)
    gate = _rb(jax.nn.sigmoid(_rb(rsel)))[:, 0:1]
    upd = mod_s[:, 3 * M:4 * M] * (y * gate)
    for k in range(TOPK):
        ob_s[pl.ds(idxs[k], 1), :] = ob_s[pl.ds(idxs[k], 1), :] + upd[k:k + 1, :]
    g0s = [pl.multiple_of(jnp.clip(idxs[k] // GR, 0, S // GR - 1) * GR, GR) for k in range(TOPK)]
    for k in range(TOPK):
        fix_s[k] = ob_s[pl.ds(g0s[k], GR), :].astype(bf)
    for blk in range(NQ):
        out_copy(blk).wait()
    for k in range(TOPK):
        cp = pltpu.make_async_copy(fix_s.at[k], out_hbm.at[pl.ds(g0s[k], GR)], sem_o.at[0])
        cp.start()
        cp.wait()


@jax.jit
def pallas_adaLN_cond__compressed_kv_cla__moe_arch_mod__prompt_kernel(
        A_x, A_c_kv, A_w_q, A_w_uk, A_w_uv, A_w_o, B_x, B_w_r, B_w_gate, B_w_up, B_w_down, c, w_mod):
    V = pltpu.VMEM
    scratch = [
        V((S, M), bf), V((S, C), bf), V((S // 2, C), u32), V((S, M), bf),
        V((2, M, D), u32), V((2, C, D), u32), V((2, C, D), u32),
        V((2, S, D), bf), V((2, S, D), bf), V((2, S, D), bf), V((2, S, D), bf),
        V((2, S, D), f32), V((H, S, D), bf),
        V((H * D, M), bf), V((M,), bf), V((FP, M), bf), V((FP, M), bf), V((FP, M), bf),
        V((2, NQ - 1, M, TQ), bf),
        V((1, M), bf), V((M, T), f32), V((M, 6 * M), bf), V((8, 5 * M), f32),
        V((TQ, M), f32), V((S, M), f32), V((S, M), f32), V((S, M), bf),
        V((8, T), f32), V((TOPK, GR, M), bf), V((2, 16, 2 * T), bf),
        pltpu.SemaphoreType.DMA((2, 3)), pltpu.SemaphoreType.DMA((len(CCH),)), pltpu.SemaphoreType.DMA((len(XCH),)),
        pltpu.SemaphoreType.DMA((8,)), pltpu.SemaphoreType.DMA((NQ,)), pltpu.SemaphoreType.REGULAR,
    ] + [V((TQ, (i + 1) * TQ), f32) for _ in range(2) for i in range(NQ)]
    out = pl.pallas_call(
        _kernel,
        in_specs=[pl.BlockSpec(memory_space=pltpu.HBM)] * 12,
        out_specs=pl.BlockSpec(memory_space=pltpu.HBM),
        out_shape=jax.ShapeDtypeStruct((S, M), bf),
        scratch_shapes=scratch,
        compiler_params=pltpu.CompilerParams(vmem_limit_bytes=124 * 1024 * 1024, disable_bounds_checks=True,
                                             disable_semaphore_checks=True),
    )(A_x.reshape(S, M), A_c_kv.reshape(S, C), A_w_q, A_w_uk, A_w_uv, A_w_o.reshape(H * D, M),
      B_w_r, B_w_gate.T, B_w_up.T, B_w_down, c, w_mod)
    return out.reshape(1, S, M)
```

```python
import jax
import jax.numpy as jnp
from jax import lax
import jax.experimental.pallas as pl
import jax.experimental.pallas.tpu as pltpu

S, M, C, H, D, F, TOPK = 2048, 640, 512, 32, 128, 1728, 8
NP = H // 2
T = 128
TQ = 256
NQ = S // TQ
HS = 64
NS = S // HS
FP = 1792
PC = 512
FR = 16
GR = 8
PAR_N = 6
LK = 8
NURG = 32
CCH = [(0, 256), (256, 768), (768, 2048)]
XCH = [(1792, 2048), (1536, 1792), (0, 1536)]
K1 = 896
K2 = 1536
K3 = 1920
VS = 1536
OS = 4
MODG = 8
MDEL = 1400
bf = jnp.bfloat16
f32 = jnp.float32
u32 = jnp.uint32
i32 = jnp.int32
NT = (((1,), (1,)), ((), ()))
EPS = 1e-5
QSCALE = D ** -0.5 * 1.4426950408889634
NEG = -1e30
KOFF = 0x10000000
KHALF = 1 << 18


def _rb(x):
    return x.astype(bf).astype(f32)


def _dot(a, b):
    return jnp.dot(a, b, preferred_element_type=f32)


def _bits(x, dt):
    return lax.bitcast_convert_type(x, dt)


def _recip(x):
    r = pl.reciprocal(x, approx=True)
    return r * (2.0 - x * r)


def _zero_after(v):
    return jnp.where(v < 0.0, 1.0, 0.0)


def _rowwise(x, w8, op):
    r, n = x.shape
    return op(x.reshape(r // 8, 8, n), w8[None]).reshape(r, n)


def _fold(x):
    n = x.shape[1] // T
    parts = [x[:, t * T:(t + 1) * T] for t in range(n)]
    nacc = 2 if n >= 4 else 1
    accs = parts[:nacc]
    for t in range(nacc, n):
        accs[t % nacc] = accs[t % nacc] + parts[t]
    return accs[0] if nacc == 1 else accs[0] + accs[1]


def _tile_lanes(v, n):
    return jnp.concatenate([v] * n, axis=1)


def _unpack_pair(w):
    lo = _bits(w << 16, f32)
    hi = _bits(w & jnp.uint32(0xFFFF0000), f32)
    return jnp.concatenate([lo, hi], axis=1).astype(bf)


def _top8(keys):
    keys = keys.reshape(keys.shape[0] // 8, 8, T)
    sub = lax.broadcasted_iota(i32, (8, T), 0)
    top = jnp.zeros((8, T), f32)
    for k in range(TOPK):
        mx = jnp.max(jnp.max(keys, axis=0), axis=0, keepdims=True)
        top = jnp.where(sub == k, mx, top)
        if k + 1 < TOPK:
            keys = jnp.where(keys == mx[None], 0.0, keys)
    return top


def _kernel(x_hbm, c_hbm, wq_hbm, wk_hbm, wv_hbm, wo_hbm, wr_hbm, wg_hbm, wu_hbm, wd_hbm, cv_hbm, wm_hbm,
            out_hbm,
            x_s, c_s, cp_s, h_s, hp_s, rq_s, rk_s, rv_s, q_s, k0_s, k_s, v_s, m_s, ctx_s,
            wo_s, wr_s, wg_s, wu_s, wd_s, wt_s, cv_s, sc_s, wm_s, mod_s, att_s, h2_s, ob_s, out_s,
            key_s, fix_s, tk_s,
            sem_w, sem_c, sem_x, sem_m, sem_o, sem_b, *s_s):
    def w_copy(w_hbm, dst, sem_col, pair, slot):
        return pltpu.make_async_copy(w_hbm.bitcast(u32).at[:, pair, :], dst.at[slot], sem_w.at[slot, sem_col])

    def step_copies(j, par):
        return [w_copy(wq_hbm, rq_s, 2, j + 1, 1 - par), w_copy(wv_hbm, rv_s, 1, j + 1, 1 - par),
                w_copy(wk_hbm, rk_s, 0, jnp.minimum(j + 2, NP - 1), par)]

    c_cp = [pltpu.make_async_copy(c_hbm.at[pl.ds(a, b - a)], c_s.at[pl.ds(a, b - a)], sem_c.at[i])
            for i, (a, b) in enumerate(CCH)]
    x_cp = [pltpu.make_async_copy(x_hbm.at[pl.ds(a, b - a)], x_s.at[pl.ds(a, b - a)], sem_x.at[i])
            for i, (a, b) in enumerate(XCH)]
    cv_cp = pltpu.make_async_copy(cv_hbm, cv_s, sem_m.at[0])
    wm0_cp = pltpu.make_async_copy(wm_hbm.at[:, pl.ds(0, 2 * M)], wm_s.at[:, pl.ds(0, 2 * M)], sem_m.at[1])
    late_cp = [pltpu.make_async_copy(wm_hbm.at[:, pl.ds(2 * M, 4 * M)], wm_s.at[:, pl.ds(2 * M, 4 * M)], sem_m.at[2]),
               pltpu.make_async_copy(wo_hbm, wo_s, sem_m.at[3]),
               pltpu.make_async_copy(wr_hbm, wr_s, sem_m.at[4]),
               pltpu.make_async_copy(wg_hbm, wg_s.at[pl.ds(0, F)], sem_m.at[5]),
               pltpu.make_async_copy(wu_hbm, wu_s.at[pl.ds(0, F)], sem_m.at[6]),
               pltpu.make_async_copy(wd_hbm, wd_s.at[pl.ds(0, F)], sem_m.at[7])]

    def out_copy(blk):
        r0 = pl.multiple_of(blk * TQ, TQ)
        return pltpu.make_async_copy(out_s.at[pl.ds(r0, TQ)], out_hbm.at[pl.ds(r0, TQ)], sem_o.at[blk])

    def fence():
        pl.semaphore_signal(sem_b, 1)
        pl.semaphore_wait(sem_b, 1)

    def urgent(z, par=None):
        src = 0 if par is None else 1 - par
        dst = 0 if par is None else par
        for _ in range(NURG):
            tk_s[dst, 0:8, 0:T] = z.astype(bf)
            z = tk_s[src, 0:8, 0:T].astype(f32)
        return z

    def proj(lhs, w, dst, a, b):
        y = _dot(lhs, w)
        dst[0, a:b, :] = y[:, 0:D].astype(bf)
        dst[1, a:b, :] = y[:, D:2 * D].astype(bf)

    def c_rows(a, b):
        return pltpu.bitcast(cp_s[a // 2:b // 2, :], bf)

    lane = lax.broadcasted_iota(i32, (HS, T), 1)
    srow = lax.broadcasted_iota(i32, (HS, T), 0)
    diag = lane <= srow + HS
    half = [lane < HS, lane >= HS]
    first = [lane <= srow, jnp.logical_and(lane >= HS, lane - HS <= srow)]

    def q_rows(e, strips):
        return jnp.concatenate([q_s[e, HS * u:HS * (u + 1), :] for u in strips], axis=0)

    def left_scores(strips, kref):
        st = [lax.dot_general(kref[e, 0:HS, :], q_rows(e, strips), NT, preferred_element_type=f32) for e in range(2)]
        return jnp.concatenate(st, axis=0).T

    def qk(e, strips, kref, left=None):
        off = HS * (1 - strips[0] % 2)
        n0 = (strips[0] + 1) // 2
        q = q_rows(e, strips)
        parts = [[] for _ in strips]
        if n0 > 0:
            s = lax.dot_general(q, kref[e, off:off + n0 * T, :], NT, preferred_element_type=f32)
            for k in range(len(strips)):
                parts[k] += [s[HS * k:HS * (k + 1), t * T:(t + 1) * T] for t in range(n0)]
        for k0 in range(1, len(strips)):
            t = n0 + k0 - 1
            s = lax.dot_general(q[HS * k0:], kref[e, off + t * T:off + (t + 1) * T, :], NT, preferred_element_type=f32)
            for k in range(k0, len(strips)):
                parts[k].append(s[HS * (k - k0):HS * (k - k0 + 1), :])
        for k, u in enumerate(strips):
            if parts[k]:
                parts[k][-1] = jnp.where(diag, parts[k][-1], NEG)
            if u % 2 == 0:
                parts[k].insert(0, jnp.where(first[e] if u == 0 else half[e], left[HS * k:HS * (k + 1), :], NEG))
            su = jnp.concatenate(parts[k], axis=1)
            s_s[e * NS + u][...] = su
            m_s[e, HS * u:HS * (u + 1), :] = jnp.broadcast_to(jnp.max(su, axis=1, keepdims=True), (HS, D))

    groups = [[8 * b + par + 2 * k for k in range(4)] for b in range(NS // 8 - 1, -1, -1) for par in (1, 0)]

    def scores(kref):
        lefts = {}
        for e in range(2):
            for g in groups:
                if g[0] % 2 and g[0] - 1 not in lefts:
                    lefts[g[0] - 1] = left_scores([u - 1 for u in g], kref)
                qk(e, g, kref, None if g[0] % 2 else lefts[g[0]])

    def softmax(tok):
        P = {}
        for e in range(2):
            for g in groups:
                for u in g:
                    P[(e, u)] = []
                    n = u // 2 + 1
                    prev = None
                    for rr in range(0, HS, 8):
                        r = HS * u + rr
                        m = m_s[e, r:r + 8, :] + tok
                        p = jnp.exp2(s_s[e * NS + u][rr:rr + 8, :] - _tile_lanes(m, n))
                        acc = _fold(p)
                        P[(e, u)].append((p, acc))
                        if n > PAR_N:
                            tok = _zero_after(acc)
                        elif prev is None:
                            prev = acc
                        else:
                            tok = _zero_after(acc + prev)
                            prev = None
        return P, tok

    def values(e, pair, P):
        for g in groups:
            n0 = g[0] // 2 + 1
            ps = [jnp.concatenate([x[0] for x in P[(e, u)]], axis=0) for u in g]

            def vt(t0, t1):
                if g[0] % 2:
                    return v_s[e, t0 * T:t1 * T, :]
                if t0 > 0:
                    return v_s[e, t0 * T - HS:t1 * T - HS, :]
                vl = [v_s[0, 0:HS, :], v_s[1, 0:HS, :]]
                return jnp.concatenate(vl + ([v_s[e, HS:t1 * T - HS, :]] if t1 > 1 else []), axis=0)

            ctx = _dot(jnp.concatenate([x[:, 0:n0 * T] for x in ps], axis=0).astype(bf), vt(0, n0))
            cs = [ctx[HS * k:HS * (k + 1)] for k in range(len(g))]
            for k0 in range(1, len(g)):
                t = n0 + k0 - 1
                c2 = _dot(jnp.concatenate([x[:, t * T:(t + 1) * T] for x in ps[k0:]], axis=0).astype(bf), vt(t, t + 1))
                for k in range(k0, len(g)):
                    cs[k] = cs[k] + c2[HS * (k - k0):HS * (k - k0 + 1)]
            for k, u in enumerate(g):
                l = jnp.sum(jnp.concatenate([x[1] for x in P[(e, u)]], axis=0), axis=1, keepdims=True)
                ctx_s[2 * pair + e, HS * u:HS * (u + 1), :] = (cs[k] * _recip(l)).astype(bf)

    def ln1(i, tok):
        starts = list(range(XCH[i][1] - 8, XCH[i][0] - 1, -8))
        nu = len(starts)
        mean, rinv = {}, {}
        for t in range(nu + 2 * LK):
            if t < nu:
                a = starts[t]
                s1 = _fold(x_s[a:a + 8, :].astype(f32)) + tok
                mean[t] = jnp.sum(s1, axis=1, keepdims=True) * (1.0 / M)
                tok = _zero_after(s1 * s1)
            u = t - LK
            if 0 <= u < nu:
                a = starts[u]
                xc = x_s[a:a + 8, :].astype(f32) - _tile_lanes(mean[u] + tok, M // T)
                s2 = _fold(xc * xc)
                rinv[u] = lax.rsqrt(jnp.sum(s2, axis=1, keepdims=True) * (1.0 / M) + EPS)
                tok = _zero_after(s2)
            u = t - 2 * LK
            if 0 <= u < nu:
                a = starts[u]
                xn = (x_s[a:a + 8, :].astype(f32) - mean[u]) * _tile_lanes(rinv[u] + tok, M // T)
                hv = xn * mod_s[:, 0:M] + mod_s[:, M:2 * M]
                h_s[a:a + 8, :] = hv.astype(bf)
                z = _fold(hv)
                tok = _zero_after(z * z)
        return urgent(tok)

    wk0_cp, wv0_cp, wq0_cp = w_copy(wk_hbm, rk_s, 0, 0, 0), w_copy(wv_hbm, rv_s, 1, 0, 0), w_copy(wq_hbm, rq_s, 2, 0, 0)
    wk1_cp = w_copy(wk_hbm, rk_s, 0, 1, 1)
    for cp in [cv_cp, wk0_cp, c_cp[0], wv0_cp, c_cp[1], wk1_cp, c_cp[2], wm0_cp, x_cp[0], wq0_cp] + x_cp[1:]:
        cp.start()
        fence()

    tok = jnp.zeros((8, T), f32)
    for w_ in (wg_s, wu_s, wd_s):
        w_[F:FP, :] = jnp.zeros((FP - F, M), bf)
    tk_s[...] = jnp.zeros(tk_s.shape, bf)
    cv_cp.wait()
    cvec = cv_s[...].astype(f32)
    silu_c = _rb(cvec * jax.nn.sigmoid(cvec))
    sc_s[...] = jnp.broadcast_to(silu_c, (T, M)).T
    wk0_cp.wait(); c_cp[0].wait(); wv0_cp.wait()
    wk0 = _unpack_pair(rk_s[0])
    wv0 = _unpack_pair(rv_s[0])

    def kv0(a, b):
        lhs = c_s[a:b, :]
        cp_s[a // 2:b // 2, :] = pltpu.bitcast(lhs, u32)
        proj(lhs, wk0, k0_s, a, b)
        proj(lhs, wv0, v_s, a, b)

    kv0(*CCH[0])
    c_cp[1].wait()
    kv0(*CCH[1])
    wk1_cp.wait()
    wk1 = _unpack_pair(rk_s[1])

    def k1(a, b):
        proj(c_s[a:b, :], wk1, k_s, a, b)

    k1(0, CCH[2][0])
    c_cp[2].wait()
    kv0(*CCH[2])
    k1(CCH[2][0], K1)
    wm0_cp.wait(); x_cp[0].wait()
    mod0 = _rb(_dot(jnp.broadcast_to(silu_c.astype(bf), (8, M)), wm_s[:, 0:2 * M]))
    mod_s[:, 0:M] = _rb(1.0 + mod0[:, M:2 * M]) * QSCALE
    mod_s[:, M:2 * M] = mod0[:, 0:M] * QSCALE
    k1(K1, K2)
    tok = ln1(0, tok)
    wq0_cp.wait(); x_cp[1].wait()
    wq0 = _unpack_pair(rq_s[0])

    def q0(i):
        lhs = h_s[i * TQ:(i + 1) * TQ, :]
        hp_s[i * TQ // 2:(i + 1) * TQ // 2, :] = pltpu.bitcast(lhs, u32)
        proj(lhs, wq0, q_s, i * TQ, (i + 1) * TQ)

    lefts = {}

    def qk0(e, i):
        if i not in lefts:
            lefts[i] = left_scores([4 * i, 4 * i + 2], k0_s)
        qk(e, [4 * i + 1, 4 * i + 3], k0_s)
        qk(e, [4 * i, 4 * i + 2], k0_s, lefts[i])

    tok = ln1(1, tok)
    q0(7); k1(K2, K2 + T); qk0(0, 7); q0(6); qk0(1, 7); k1(K2 + T, K2 + 2 * T)
    for cp in step_copies(0, 0):
        cp.start()
    for cp in late_cp:
        cp.start(priority=1)
    x_cp[2].wait()
    tok = ln1(2, tok)
    qk0(0, 6); qk0(1, 6)
    q0(5)
    k1(K2 + 2 * T, K3)
    qk0(0, 5); q0(4); qk0(1, 5); qk0(0, 4); q0(3); qk0(1, 4); qk0(0, 3); q0(2)
    q0(1); qk0(0, 2); q0(0); qk0(1, 2)
    qk0(0, 1); qk0(1, 1); qk0(0, 0); qk0(1, 0); qk0(1, 3)
    k1(K3, S)

    def late_mod(tok):
        for _ in range(MDEL):
            tok = tok * tok
        cols = []
        for jt in range(4 * M // T):
            w = wm_s[:, 2 * M + jt * T:2 * M + (jt + 1) * T].astype(f32)
            acc = None
            for g in range(M // 8):
                t_ = (w[8 * g:8 * g + 8, :] + tok) * sc_s[8 * g:8 * g + 8, :]
                acc = t_ if acc is None else acc + t_
                if (g + 1) % MODG == 0:
                    tok = _zero_after(acc * acc)
            cols.append(jnp.broadcast_to(jnp.sum(acc, axis=0, keepdims=True), (8, T)))
        mod1 = _rb(jnp.concatenate(cols, axis=1))
        mod_s[:, 0:2 * M] = mod1[:, 0:2 * M]
        mod_s[:, 2 * M:3 * M] = _rb(1.0 + mod1[:, 2 * M:3 * M])
        mod_s[:, 3 * M:4 * M] = mod1[:, 3 * M:4 * M]
        mod_s[:, 4 * M:5 * M] = jnp.broadcast_to(wr_s[...].astype(f32).reshape(1, M), (8, M))
        return tok

    def step(j, tok, last):
        par = j & 1
        for cp in step_copies(j, par):
            cp.wait()
        P, tok = softmax(tok)
        if last:
            tok = late_mod(tok)
        wq = _unpack_pair(rq_s[1 - par])
        if not last:
            for cp in step_copies(j + 1, 1 - par):
                cp.start()
        for a in range(0, S, PC):
            proj(pltpu.bitcast(hp_s[a // 2:(a + PC) // 2, :], bf), wq, q_s, a, a + PC)

        wv = _unpack_pair(rv_s[1 - par])

        def vproj(lo, hi):
            for a in range(lo, hi, PC):
                proj(c_rows(a, a + PC), wv, v_s, a, a + PC)

        values(0, j, P)
        values(1, j, P)
        vproj(0, VS if last else S)
        scores(k_s)
        if last:
            vproj(VS, S)
        else:
            wk = _unpack_pair(rk_s[par])
            for a in range(S - PC, -1, -PC):
                proj(c_rows(a, a + PC), wk, k_s, a, a + PC)
        return urgent(tok, None if last else par)
    tok = lax.fori_loop(0, NP - 2, lambda j, t: step(j, t, False), tok)
    late_cp[0].wait(); late_cp[2].wait()
    tok = step(NP - 2, tok, True)

    for cp in late_cp[1:2] + late_cp[3:]:
        cp.wait()

    def oproj(r0, h0, h1):
        lhs = jnp.concatenate([ctx_s[h, pl.ds(r0, TQ), :] for h in range(h0, h1)], axis=1)
        return _dot(lhs, wo_s[h0 * D:h1 * D, :])

    P, tok = softmax(tok)
    att_s[...] = oproj((NQ - 1) * TQ, 0, H - OS)
    values(0, NP - 1, P)
    values(1, NP - 1, P)
    att_s[...] += oproj((NQ - 1) * TQ, H - OS, H)
    key_s[...] = urgent(tok)

    def finish(blk, paced):
        r0 = pl.multiple_of(blk * TQ, TQ)
        ga, sb, cb1, gb, wr = [mod_s[:, k * M:(k + 1) * M] for k in range(5)]
        tok = None
        keys = [key_s[...]]
        for a in range(0, TQ, FR):
            ra = pl.multiple_of(r0 + a, FR)
            x1 = x_s[pl.ds(ra, FR), :].astype(f32) + _rowwise(att_s[a:a + FR, :], ga, jnp.multiply)
            m = jnp.sum(x1, axis=1, keepdims=True) * (1.0 / M)
            if tok is not None:
                m = m + tok
            xc = x1 - m
            rinv = lax.rsqrt(jnp.sum(xc * xc, axis=1, keepdims=True) * (1.0 / M) + EPS)
            h2 = _rowwise(_rowwise(xc * rinv, cb1, jnp.multiply), sb, jnp.add)
            h2_s[pl.ds(ra, FR), :] = h2
            ob = x1 + _rowwise(h2, gb, jnp.multiply)
            ob_s[pl.ds(ra, FR), :] = ob
            out_s[pl.ds(ra, FR), :] = ob.astype(bf)
            r = jnp.sum(_rowwise(h2, wr, jnp.multiply), axis=1, keepdims=True) + 0.0
            if paced:
                tok = _zero_after(r * r)
            b = _bits(jnp.broadcast_to(r, (FR, T)), i32) >> 13
            o = jnp.where(b < 0, (KHALF - 1) - (b & (KHALF - 1)), b + KHALF)
            rws = lax.broadcasted_iota(i32, (FR, T), 0) + ra
            keys.append(_bits((o << 11) + (KOFF + S - 1 - rws), f32))
            if paced or a + FR == TQ:
                keys = [_top8(jnp.concatenate(keys, axis=0))]
        key_s[...] = keys[0]
        out_copy(blk).start()

    def oblock(t, carry):
        blk = NQ - 2 - t
        finish(blk + 1, True)
        f0 = pl.multiple_of(t * TQ, TQ)
        wt_s[0, t] = wg_s[pl.ds(f0, TQ), :].T
        wt_s[1, t] = wu_s[pl.ds(f0, TQ), :].T
        att_s[...] = oproj(pl.multiple_of(blk * TQ, TQ), 0, H)
        return carry
    lax.fori_loop(0, NQ - 1, oblock, 0)
    finish(0, False)

    sel = _bits(key_s[...], i32)
    rowid = (S - 1) - (sel & (S - 1))
    idxs = [jnp.clip(rowid[k, 0], 0, S - 1) for k in range(TOPK)]
    xs = jnp.concatenate([h2_s[pl.ds(ix, 1), :] for ix in idxs], axis=0).astype(bf)
    g = _rb(_dot(xs, jnp.concatenate([wt_s[0, t] for t in range(NQ - 1)], axis=1)))
    g = _rb(g * jax.nn.sigmoid(g))
    u = _rb(_dot(xs, jnp.concatenate([wt_s[1, t] for t in range(NQ - 1)], axis=1)))
    y = _rb(_dot((g * u).astype(bf), wd_s[...]))
    o = (sel - KOFF) >> 11
    rsel = _bits((jnp.where(o >= KHALF, o - KHALF, 2 * KHALF - 1 - o) << 13) | 4096, f32)
    gate = _rb(jax.nn.sigmoid(_rb(rsel)))[:, 0:1]
    upd = mod_s[:, 3 * M:4 * M] * (y * gate)
    for k in range(TOPK):
        ob_s[pl.ds(idxs[k], 1), :] = ob_s[pl.ds(idxs[k], 1), :] + upd[k:k + 1, :]
    g0s = [pl.multiple_of(jnp.clip(idxs[k] // GR, 0, S // GR - 1) * GR, GR) for k in range(TOPK)]
    for k in range(TOPK):
        fix_s[k] = ob_s[pl.ds(g0s[k], GR), :].astype(bf)
    for blk in range(NQ):
        out_copy(blk).wait()
    for k in range(TOPK):
        cp = pltpu.make_async_copy(fix_s.at[k], out_hbm.at[pl.ds(g0s[k], GR)], sem_o.at[0])
        cp.start()
        cp.wait()


@jax.jit
def pallas_adaLN_cond__compressed_kv_cla__moe_arch_mod__prompt_kernel(
        A_x, A_c_kv, A_w_q, A_w_uk, A_w_uv, A_w_o, B_x, B_w_r, B_w_gate, B_w_up, B_w_down, c, w_mod):
    V = pltpu.VMEM
    scratch = [
        V((S, M), bf), V((S, C), bf), V((S // 2, C), u32), V((S, M), bf), V((S // 2, M), u32),
        V((2, M, D), u32), V((2, C, D), u32), V((2, C, D), u32),
        V((2, S, D), bf), V((2, S, D), bf), V((2, S, D), bf), V((2, S, D), bf),
        V((2, S, D), f32), V((H, S, D), bf),
        V((H * D, M), bf), V((M,), bf), V((FP, M), bf), V((FP, M), bf), V((FP, M), bf),
        V((2, NQ - 1, M, TQ), bf),
        V((1, M), bf), V((M, T), f32), V((M, 6 * M), bf), V((8, 5 * M), f32),
        V((TQ, M), f32), V((S, M), f32), V((S, M), f32), V((S, M), bf),
        V((8, T), f32), V((TOPK, GR, M), bf), V((2, 16, 2 * T), bf),
        pltpu.SemaphoreType.DMA((2, 3)), pltpu.SemaphoreType.DMA((len(CCH),)), pltpu.SemaphoreType.DMA((len(XCH),)),
        pltpu.SemaphoreType.DMA((8,)), pltpu.SemaphoreType.DMA((NQ,)), pltpu.SemaphoreType.REGULAR,
    ] + [V((HS, (u // 2 + 1) * T), f32) for _ in range(2) for u in range(NS)]
    out = pl.pallas_call(
        _kernel,
        in_specs=[pl.BlockSpec(memory_space=pltpu.HBM)] * 12,
        out_specs=pl.BlockSpec(memory_space=pltpu.HBM),
        out_shape=jax.ShapeDtypeStruct((S, M), bf),
        scratch_shapes=scratch,
        compiler_params=pltpu.CompilerParams(vmem_limit_bytes=124 * 1024 * 1024, disable_bounds_checks=True,
                                             disable_semaphore_checks=True),
    )(A_x.reshape(S, M), A_c_kv.reshape(S, C), A_w_q, A_w_uk, A_w_uv, A_w_o.reshape(H * D, M),
      B_w_r, B_w_gate.T, B_w_up.T, B_w_down, c, w_mod)
    return out.reshape(1, S, M)
```

```python
import jax
import jax.numpy as jnp
from jax import lax
import jax.experimental.pallas as pl
import jax.experimental.pallas.tpu as pltpu

S, M, C, H, D, F, TOPK = 2048, 640, 512, 32, 128, 1728, 8
NP = H // 2
T = 128
TQ = 256
NQ = S // TQ
HS = 64
NS = S // HS
FP = 1792
PC = 512
FR = 16
GR = 8
PAR_N = 6
LK = 8
NURG = 32
CCH = [(0, 256), (256, 768), (768, 2048)]
XCH = [(1792, 2048), (1536, 1792), (0, 1536)]
K1 = 896
K2 = 1536
K3 = 1920
VS = 1536
OS = 4
MODG = 8
MDEL = 1400
bf = jnp.bfloat16
f32 = jnp.float32
u32 = jnp.uint32
i32 = jnp.int32
NT = (((1,), (1,)), ((), ()))
EPS = 1e-5
QSCALE = D ** -0.5 * 1.4426950408889634
NEG = -1e30
KOFF = 0x10000000
KHALF = 1 << 18


def _rb(x):
    return x.astype(bf).astype(f32)


def _dot(a, b):
    return jnp.dot(a, b, preferred_element_type=f32)


def _bits(x, dt):
    return lax.bitcast_convert_type(x, dt)


def _recip(x):
    r = pl.reciprocal(x, approx=True)
    return r * (2.0 - x * r)


def _zero_after(v):
    return jnp.where(v < 0.0, 1.0, 0.0)


def _rowwise(x, w8, op):
    r, n = x.shape
    return op(x.reshape(r // 8, 8, n), w8[None]).reshape(r, n)


def _fold(x):
    n = x.shape[1] // T
    parts = [x[:, t * T:(t + 1) * T] for t in range(n)]
    nacc = 2 if n >= 4 else 1
    accs = parts[:nacc]
    for t in range(nacc, n):
        accs[t % nacc] = accs[t % nacc] + parts[t]
    return accs[0] if nacc == 1 else accs[0] + accs[1]


def _tile_lanes(v, n):
    return jnp.concatenate([v] * n, axis=1)


def _unpack_pair(w):
    lo = _bits(w << 16, f32)
    hi = _bits(w & jnp.uint32(0xFFFF0000), f32)
    return jnp.concatenate([lo, hi], axis=1).astype(bf)


def _top8(keys):
    keys = keys.reshape(keys.shape[0] // 8, 8, T)
    sub = lax.broadcasted_iota(i32, (8, T), 0)
    top = jnp.zeros((8, T), f32)
    for k in range(TOPK):
        mx = jnp.max(jnp.max(keys, axis=0), axis=0, keepdims=True)
        top = jnp.where(sub == k, mx, top)
        if k + 1 < TOPK:
            keys = jnp.where(keys == mx[None], 0.0, keys)
    return top


def _kernel(x_hbm, c_hbm, wq_hbm, wk_hbm, wv_hbm, wo_hbm, wr_hbm, wg_hbm, wu_hbm, wd_hbm, cv_hbm, wm_hbm,
            out_hbm,
            x_s, c_s, cp_s, h_s, hp_s, rq_s, rk_s, rv_s, q_s, k0_s, k_s, v_s, m_s, ctx_s,
            wo_s, wr_s, wg_s, wu_s, wd_s, wt_s, cv_s, sc_s, wm_s, mod_s, att_s, h2_s, ob_s, out_s,
            key_s, fix_s, tk_s,
            sem_w, sem_c, sem_x, sem_m, sem_o, sem_b, *s_s):
    def w_copy(w_hbm, dst, sem_col, pair, slot):
        return pltpu.make_async_copy(w_hbm.bitcast(u32).at[:, pair, :], dst.at[slot], sem_w.at[slot, sem_col])

    def step_copies(j, par):
        return [w_copy(wq_hbm, rq_s, 2, j + 1, 1 - par), w_copy(wv_hbm, rv_s, 1, j + 1, 1 - par),
                w_copy(wk_hbm, rk_s, 0, jnp.minimum(j + 2, NP - 1), par)]

    c_cp = [pltpu.make_async_copy(c_hbm.at[pl.ds(a, b - a)], c_s.at[pl.ds(a, b - a)], sem_c.at[i])
            for i, (a, b) in enumerate(CCH)]
    x_cp = [pltpu.make_async_copy(x_hbm.at[pl.ds(a, b - a)], x_s.at[pl.ds(a, b - a)], sem_x.at[i])
            for i, (a, b) in enumerate(XCH)]
    cv_cp = pltpu.make_async_copy(cv_hbm, cv_s, sem_m.at[0])
    wm0_cp = pltpu.make_async_copy(wm_hbm.at[:, pl.ds(0, 2 * M)], wm_s.at[:, pl.ds(0, 2 * M)], sem_m.at[1])
    late_cp = [pltpu.make_async_copy(wm_hbm.at[:, pl.ds(2 * M, 4 * M)], wm_s.at[:, pl.ds(2 * M, 4 * M)], sem_m.at[2]),
               pltpu.make_async_copy(wo_hbm, wo_s, sem_m.at[3]),
               pltpu.make_async_copy(wr_hbm, wr_s, sem_m.at[4]),
               pltpu.make_async_copy(wg_hbm, wg_s.at[pl.ds(0, F)], sem_m.at[5]),
               pltpu.make_async_copy(wu_hbm, wu_s.at[pl.ds(0, F)], sem_m.at[6]),
               pltpu.make_async_copy(wd_hbm, wd_s.at[pl.ds(0, F)], sem_m.at[7])]

    def out_copy(blk):
        r0 = pl.multiple_of(blk * TQ, TQ)
        return pltpu.make_async_copy(out_s.at[pl.ds(r0, TQ)], out_hbm.at[pl.ds(r0, TQ)], sem_o.at[blk])

    def fence():
        pl.semaphore_signal(sem_b, 1)
        pl.semaphore_wait(sem_b, 1)

    def urgent(z, par=None):
        src = 0 if par is None else 1 - par
        dst = 0 if par is None else par
        for _ in range(NURG):
            tk_s[dst, 0:8, 0:T] = z.astype(bf)
            z = tk_s[src, 0:8, 0:T].astype(f32)
        return z

    def proj(lhs, w, dst, a, b):
        y = _dot(lhs, w)
        dst[0, a:b, :] = y[:, 0:D].astype(bf)
        dst[1, a:b, :] = y[:, D:2 * D].astype(bf)

    def c_rows(a, b):
        return pltpu.bitcast(cp_s[a // 2:b // 2, :], bf)

    lane = lax.broadcasted_iota(i32, (HS, T), 1)
    srow = lax.broadcasted_iota(i32, (HS, T), 0)
    diag = lane <= srow + HS
    half = [lane < HS, lane >= HS]
    first = [lane <= srow, jnp.logical_and(lane >= HS, lane - HS <= srow)]

    def q_rows(e, strips):
        return jnp.concatenate([q_s[e, HS * u:HS * (u + 1), :] for u in strips], axis=0)

    def left_scores(strips, kref):
        st = [lax.dot_general(kref[e, 0:HS, :], q_rows(e, strips), NT, preferred_element_type=f32) for e in range(2)]
        return jnp.concatenate(st, axis=0).T

    def qk(e, strips, kref, left=None):
        off = HS * (1 - strips[0] % 2)
        n0 = (strips[0] + 1) // 2
        q = q_rows(e, strips)
        parts = [[] for _ in strips]
        if n0 > 0:
            s = lax.dot_general(q, kref[e, off:off + n0 * T, :], NT, preferred_element_type=f32)
            for k in range(len(strips)):
                parts[k] += [s[HS * k:HS * (k + 1), t * T:(t + 1) * T] for t in range(n0)]
        for k0 in range(1, len(strips)):
            t = n0 + k0 - 1
            s = lax.dot_general(q[HS * k0:], kref[e, off + t * T:off + (t + 1) * T, :], NT, preferred_element_type=f32)
            for k in range(k0, len(strips)):
                parts[k].append(s[HS * (k - k0):HS * (k - k0 + 1), :])
        for k, u in enumerate(strips):
            if parts[k]:
                parts[k][-1] = jnp.where(diag, parts[k][-1], NEG)
            if u % 2 == 0:
                parts[k].insert(0, jnp.where(first[e] if u == 0 else half[e], left[HS * k:HS * (k + 1), :], NEG))
            su = jnp.concatenate(parts[k], axis=1)
            s_s[e * NS + u][...] = su
            m_s[e, HS * u:HS * (u + 1), :] = jnp.broadcast_to(jnp.max(su, axis=1, keepdims=True), (HS, D))

    groups = [[8 * b + par + 2 * k for k in range(4)] for b in range(NS // 8 - 1, -1, -1) for par in (1, 0)]

    def scores(kref):
        lefts = {}
        for e in range(2):
            for g in groups:
                if g[0] % 2 and g[0] - 1 not in lefts:
                    lefts[g[0] - 1] = left_scores([u - 1 for u in g], kref)
                qk(e, g, kref, None if g[0] % 2 else lefts[g[0]])

    def softmax(tok):
        P = {}
        for e in range(2):
            for g in groups:
                for u in g:
                    P[(e, u)] = []
                    n = u // 2 + 1
                    prev = None
                    for rr in range(0, HS, 8):
                        r = HS * u + rr
                        m = m_s[e, r:r + 8, :] + tok
                        p = jnp.exp2(s_s[e * NS + u][rr:rr + 8, :] - _tile_lanes(m, n))
                        acc = _fold(p)
                        P[(e, u)].append((p, acc))
                        if n > PAR_N:
                            tok = _zero_after(acc)
                        elif prev is None:
                            prev = acc
                        else:
                            tok = _zero_after(acc + prev)
                            prev = None
        return P, tok

    def values(e, pair, P):
        for g in groups:
            n0 = g[0] // 2 + 1
            ps = [jnp.concatenate([x[0] for x in P[(e, u)]], axis=0) for u in g]

            def vt(t0, t1):
                if g[0] % 2:
                    return v_s[e, t0 * T:t1 * T, :]
                if t0 > 0:
                    return v_s[e, t0 * T - HS:t1 * T - HS, :]
                vl = [v_s[0, 0:HS, :], v_s[1, 0:HS, :]]
                return jnp.concatenate(vl + ([v_s[e, HS:t1 * T - HS, :]] if t1 > 1 else []), axis=0)

            ctx = _dot(jnp.concatenate([x[:, 0:n0 * T] for x in ps], axis=0).astype(bf), vt(0, n0))
            cs = [ctx[HS * k:HS * (k + 1)] for k in range(len(g))]
            for k0 in range(1, len(g)):
                t = n0 + k0 - 1
                c2 = _dot(jnp.concatenate([x[:, t * T:(t + 1) * T] for x in ps[k0:]], axis=0).astype(bf), vt(t, t + 1))
                for k in range(k0, len(g)):
                    cs[k] = cs[k] + c2[HS * (k - k0):HS * (k - k0 + 1)]
            for k, u in enumerate(g):
                l = jnp.sum(jnp.concatenate([x[1] for x in P[(e, u)]], axis=0), axis=1, keepdims=True)
                ctx_s[2 * pair + e, HS * u:HS * (u + 1), :] = (cs[k] * _recip(l)).astype(bf)

    def ln1(i, tok):
        starts = list(range(XCH[i][1] - 8, XCH[i][0] - 1, -8))
        nu = len(starts)
        mean, rinv = {}, {}
        for t in range(nu + 2 * LK):
            if t < nu:
                a = starts[t]
                s1 = _fold(x_s[a:a + 8, :].astype(f32)) + tok
                mean[t] = jnp.sum(s1, axis=1, keepdims=True) * (1.0 / M)
                tok = _zero_after(s1 * s1)
            u = t - LK
            if 0 <= u < nu:
                a = starts[u]
                xc = x_s[a:a + 8, :].astype(f32) - _tile_lanes(mean[u] + tok, M // T)
                s2 = _fold(xc * xc)
                rinv[u] = lax.rsqrt(jnp.sum(s2, axis=1, keepdims=True) * (1.0 / M) + EPS)
                tok = _zero_after(s2)
            u = t - 2 * LK
            if 0 <= u < nu:
                a = starts[u]
                xn = (x_s[a:a + 8, :].astype(f32) - mean[u]) * _tile_lanes(rinv[u] + tok, M // T)
                hv = xn * mod_s[:, 0:M] + mod_s[:, M:2 * M]
                h_s[a:a + 8, :] = hv.astype(bf)
                z = _fold(hv)
                tok = _zero_after(z * z)
        return urgent(tok)

    wk0_cp, wv0_cp, wq0_cp = w_copy(wk_hbm, rk_s, 0, 0, 0), w_copy(wv_hbm, rv_s, 1, 0, 0), w_copy(wq_hbm, rq_s, 2, 0, 0)
    wk1_cp = w_copy(wk_hbm, rk_s, 0, 1, 1)
    for cp in [cv_cp, wk0_cp, c_cp[0], wv0_cp, c_cp[1], wk1_cp, c_cp[2], wm0_cp, x_cp[0], wq0_cp] + x_cp[1:]:
        cp.start()
        fence()

    tok = jnp.zeros((8, T), f32)
    for w_ in (wg_s, wu_s, wd_s):
        w_[F:FP, :] = jnp.zeros((FP - F, M), bf)
    tk_s[...] = jnp.zeros(tk_s.shape, bf)
    cv_cp.wait()
    cvec = cv_s[...].astype(f32)
    silu_c = _rb(cvec * jax.nn.sigmoid(cvec))
    sc_s[...] = jnp.broadcast_to(silu_c, (T, M)).T
    wk0_cp.wait(); c_cp[0].wait(); wv0_cp.wait()
    wk0 = _unpack_pair(rk_s[0])
    wv0 = _unpack_pair(rv_s[0])

    def kv0(a, b):
        lhs = c_s[a:b, :]
        cp_s[a // 2:b // 2, :] = pltpu.bitcast(lhs, u32)
        proj(lhs, wk0, k0_s, a, b)
        proj(lhs, wv0, v_s, a, b)

    kv0(*CCH[0])
    c_cp[1].wait()
    kv0(*CCH[1])
    wk1_cp.wait()
    wk1 = _unpack_pair(rk_s[1])

    def k1(a, b):
        proj(c_s[a:b, :], wk1, k_s, a, b)

    k1(0, CCH[2][0])
    c_cp[2].wait()
    kv0(*CCH[2])
    k1(CCH[2][0], K1)
    wm0_cp.wait(); x_cp[0].wait()
    mod0 = _rb(_dot(jnp.broadcast_to(silu_c.astype(bf), (8, M)), wm_s[:, 0:2 * M]))
    mod_s[:, 0:M] = _rb(1.0 + mod0[:, M:2 * M]) * QSCALE
    mod_s[:, M:2 * M] = mod0[:, 0:M] * QSCALE
    k1(K1, K2)
    tok = ln1(0, tok)
    wq0_cp.wait(); x_cp[1].wait()
    wq0 = _unpack_pair(rq_s[0])

    def q0(i):
        lhs = h_s[i * TQ:(i + 1) * TQ, :]
        hp_s[i * TQ // 2:(i + 1) * TQ // 2, :] = pltpu.bitcast(lhs, u32)
        proj(lhs, wq0, q_s, i * TQ, (i + 1) * TQ)

    lefts = {}

    def qk0(e, i):
        if i not in lefts:
            lefts[i] = left_scores([4 * i, 4 * i + 2], k0_s)
        qk(e, [4 * i + 1, 4 * i + 3], k0_s)
        qk(e, [4 * i, 4 * i + 2], k0_s, lefts[i])

    tok = ln1(1, tok)
    q0(7); k1(K2, K2 + T); qk0(0, 7); q0(6); qk0(1, 7); k1(K2 + T, K2 + 2 * T)
    for cp in step_copies(0, 0):
        cp.start()
    for cp in late_cp:
        cp.start(priority=1)
    x_cp[2].wait()
    tok = ln1(2, tok)
    qk0(0, 6); qk0(1, 6)
    q0(5)
    k1(K2 + 2 * T, K3)
    qk0(0, 5); q0(4); qk0(1, 5); qk0(0, 4); q0(3); qk0(1, 4); qk0(0, 3); q0(2)
    q0(1); qk0(0, 2); q0(0); qk0(1, 2)
    qk0(0, 1); qk0(1, 1); qk0(0, 0); qk0(1, 0); qk0(1, 3)
    k1(K3, S)

    def late_mod(tok):
        for _ in range(MDEL):
            tok = tok * tok
        cols = []
        for jt in range(4 * M // T):
            w = wm_s[:, 2 * M + jt * T:2 * M + (jt + 1) * T].astype(f32)
            acc = None
            for g in range(M // 8):
                t_ = (w[8 * g:8 * g + 8, :] + tok) * sc_s[8 * g:8 * g + 8, :]
                acc = t_ if acc is None else acc + t_
                if (g + 1) % MODG == 0:
                    tok = _zero_after(acc * acc)
            cols.append(jnp.broadcast_to(jnp.sum(acc, axis=0, keepdims=True), (8, T)))
        mod1 = _rb(jnp.concatenate(cols, axis=1))
        mod_s[:, 0:2 * M] = mod1[:, 0:2 * M]
        mod_s[:, 2 * M:3 * M] = _rb(1.0 + mod1[:, 2 * M:3 * M])
        mod_s[:, 3 * M:4 * M] = mod1[:, 3 * M:4 * M]
        mod_s[:, 4 * M:5 * M] = jnp.broadcast_to(wr_s[...].astype(f32).reshape(1, M), (8, M))
        return tok

    def step(j, tok, last):
        par = j & 1
        for cp in step_copies(j, par):
            cp.wait()
        P, tok = softmax(tok)
        if last:
            tok = late_mod(tok)
        wq = _unpack_pair(rq_s[1 - par])
        if not last:
            for cp in step_copies(j + 1, 1 - par):
                cp.start()
        for a in range(0, S, PC):
            proj(pltpu.bitcast(hp_s[a // 2:(a + PC) // 2, :], bf), wq, q_s, a, a + PC)

        wv = _unpack_pair(rv_s[1 - par])

        def vproj(lo, hi):
            for a in range(lo, hi, PC):
                proj(c_rows(a, a + PC), wv, v_s, a, a + PC)

        values(0, j, P)
        values(1, j, P)
        vproj(0, VS if last else S)
        scores(k_s)
        if last:
            vproj(VS, S)
        else:
            wk = _unpack_pair(rk_s[par])
            for a in range(S - PC, -1, -PC):
                proj(c_rows(a, a + PC), wk, k_s, a, a + PC)
        return urgent(tok, None if last else par)
    tok = lax.fori_loop(0, NP - 2, lambda j, t: step(j, t, False), tok)
    late_cp[0].wait(); late_cp[2].wait()
    tok = step(NP - 2, tok, True)

    for cp in late_cp[1:2] + late_cp[3:]:
        cp.wait()

    def oproj(r0, h0, h1):
        lhs = jnp.concatenate([ctx_s[h, pl.ds(r0, TQ), :] for h in range(h0, h1)], axis=1)
        return _dot(lhs, wo_s[h0 * D:h1 * D, :])

    P, tok = softmax(tok)
    att_s[...] = oproj((NQ - 1) * TQ, 0, H - OS)
    values(0, NP - 1, P)
    values(1, NP - 1, P)
    att_s[...] += oproj((NQ - 1) * TQ, H - OS, H)
    key_s[...] = urgent(tok)

    def finish(blk, paced):
        r0 = pl.multiple_of(blk * TQ, TQ)
        ga, sb, cb1, gb, wr = [mod_s[:, k * M:(k + 1) * M] for k in range(5)]
        tok = None
        keys = [key_s[...]]
        for a in range(0, TQ, FR):
            ra = pl.multiple_of(r0 + a, FR)
            x1 = x_s[pl.ds(ra, FR), :].astype(f32) + _rowwise(att_s[a:a + FR, :], ga, jnp.multiply)
            m = jnp.sum(x1, axis=1, keepdims=True) * (1.0 / M)
            if tok is not None:
                m = m + tok
            xc = x1 - m
            rinv = lax.rsqrt(jnp.sum(xc * xc, axis=1, keepdims=True) * (1.0 / M) + EPS)
            h2 = _rowwise(_rowwise(xc * rinv, cb1, jnp.multiply), sb, jnp.add)
            h2_s[pl.ds(ra, FR), :] = h2
            ob = x1 + _rowwise(h2, gb, jnp.multiply)
            ob_s[pl.ds(ra, FR), :] = ob
            out_s[pl.ds(ra, FR), :] = ob.astype(bf)
            r = jnp.sum(_rowwise(h2, wr, jnp.multiply), axis=1, keepdims=True) + 0.0
            if paced:
                tok = _zero_after(r * r)
            b = _bits(jnp.broadcast_to(r, (FR, T)), i32) >> 13
            o = jnp.where(b < 0, (KHALF - 1) - (b & (KHALF - 1)), b + KHALF)
            rws = lax.broadcasted_iota(i32, (FR, T), 0) + ra
            keys.append(_bits((o << 11) + (KOFF + S - 1 - rws), f32))
            if paced or a + FR == TQ:
                keys = [_top8(jnp.concatenate(keys, axis=0))]
        key_s[...] = keys[0]
        out_copy(blk).start()

    def oblock(t, carry):
        blk = NQ - 2 - t
        finish(blk + 1, True)
        f0 = pl.multiple_of(t * TQ, TQ)
        wt_s[0, t] = wg_s[pl.ds(f0, TQ), :].T
        wt_s[1, t] = wu_s[pl.ds(f0, TQ), :].T
        att_s[...] = oproj(pl.multiple_of(blk * TQ, TQ), 0, H)
        return carry
    lax.fori_loop(0, NQ - 1, oblock, 0)
    finish(0, False)

    sel = _bits(key_s[...], i32)
    rowid = (S - 1) - (sel & (S - 1))
    idxs = [jnp.clip(rowid[k, 0], 0, S - 1) for k in range(TOPK)]
    xs = jnp.concatenate([h2_s[pl.ds(ix, 1), :] for ix in idxs], axis=0).astype(bf)
    g = _rb(_dot(xs, jnp.concatenate([wt_s[0, t] for t in range(NQ - 1)], axis=1)))
    g = _rb(g * jax.nn.sigmoid(g))
    u = _rb(_dot(xs, jnp.concatenate([wt_s[1, t] for t in range(NQ - 1)], axis=1)))
    y = _rb(_dot((g * u).astype(bf), wd_s[...]))
    o = (sel - KOFF) >> 11
    rsel = _bits((jnp.where(o >= KHALF, o - KHALF, 2 * KHALF - 1 - o) << 13) | 4096, f32)
    gate = _rb(jax.nn.sigmoid(_rb(rsel)))[:, 0:1]
    base = jnp.concatenate([ob_s[pl.ds(ix, 1), :] for ix in idxs], axis=0)
    new = base + mod_s[:, 3 * M:4 * M] * (y * gate)
    prev = None
    for k in range(TOPK):
        g0 = pl.multiple_of(jnp.clip(idxs[k] >> 3, 0, S // GR - 1) * GR, GR)
        ob_s[pl.ds(idxs[k], 1), :] = new[k:k + 1, :]
        fix_s[k] = ob_s[pl.ds(g0, GR), :].astype(bf)
        if prev is None:
            for blk in range(NQ):
                out_copy(blk).wait()
        else:
            prev.wait()
        prev = pltpu.make_async_copy(fix_s.at[k], out_hbm.at[pl.ds(g0, GR)], sem_o.at[0])
        prev.start()
        fence()
    prev.wait()


@jax.jit
def pallas_adaLN_cond__compressed_kv_cla__moe_arch_mod__prompt_kernel(
        A_x, A_c_kv, A_w_q, A_w_uk, A_w_uv, A_w_o, B_x, B_w_r, B_w_gate, B_w_up, B_w_down, c, w_mod):
    V = pltpu.VMEM
    scratch = [
        V((S, M), bf), V((S, C), bf), V((S // 2, C), u32), V((S, M), bf), V((S // 2, M), u32),
        V((2, M, D), u32), V((2, C, D), u32), V((2, C, D), u32),
        V((2, S, D), bf), V((2, S, D), bf), V((2, S, D), bf), V((2, S, D), bf),
        V((2, S, D), f32), V((H, S, D), bf),
        V((H * D, M), bf), V((M,), bf), V((FP, M), bf), V((FP, M), bf), V((FP, M), bf),
        V((2, NQ - 1, M, TQ), bf),
        V((1, M), bf), V((M, T), f32), V((M, 6 * M), bf), V((8, 5 * M), f32),
        V((TQ, M), f32), V((S, M), f32), V((S, M), f32), V((S, M), bf),
        V((8, T), f32), V((TOPK, GR, M), bf), V((2, 16, 2 * T), bf),
        pltpu.SemaphoreType.DMA((2, 3)), pltpu.SemaphoreType.DMA((len(CCH),)), pltpu.SemaphoreType.DMA((len(XCH),)),
        pltpu.SemaphoreType.DMA((8,)), pltpu.SemaphoreType.DMA((NQ,)), pltpu.SemaphoreType.REGULAR,
    ] + [V((HS, (u // 2 + 1) * T), f32) for _ in range(2) for u in range(NS)]
    out = pl.pallas_call(
        _kernel,
        in_specs=[pl.BlockSpec(memory_space=pltpu.HBM)] * 12,
        out_specs=pl.BlockSpec(memory_space=pltpu.HBM),
        out_shape=jax.ShapeDtypeStruct((S, M), bf),
        scratch_shapes=scratch,
        compiler_params=pltpu.CompilerParams(vmem_limit_bytes=124 * 1024 * 1024, disable_bounds_checks=True,
                                             disable_semaphore_checks=True),
    )(A_x.reshape(S, M), A_c_kv.reshape(S, C), A_w_q, A_w_uk, A_w_uv, A_w_o.reshape(H * D, M),
      B_w_r, B_w_gate.T, B_w_up.T, B_w_down, c, w_mod)
    return out.reshape(1, S, M)
```

```python
import jax
import jax.numpy as jnp
from jax import lax
import jax.experimental.pallas as pl
import jax.experimental.pallas.tpu as pltpu

S, M, C, H, D, F, TOPK = 2048, 640, 512, 32, 128, 1728, 8
NP = H // 2
T = 128
TQ = 256
NQ = S // TQ
HS = 64
NS = S // HS
RA, RB, NB = 256, 128, 5
FP = 1792
PC = 512
FR = 16
GR = 8
PAR_N = 6
LK = 8
NURG = 32
CCH = [(0, 256), (256, 768), (768, 2048)]
XCH = [(1792, 2048), (1536, 1792), (0, 1536)]
K1, K2, K3 = 896, 1536, 1920
VS = 1536
OS = 4
MODG = 8
MDEL = 1400
bf = jnp.bfloat16
f32 = jnp.float32
u32 = jnp.uint32
i32 = jnp.int32
NT = (((1,), (1,)), ((), ()))
EPS = 1e-5
QSCALE = D ** -0.5 * 1.4426950408889634
NEG = -1e30
KOFF = 0x10000000
KHALF = 1 << 18


def _rb(x):
    return x.astype(bf).astype(f32)


def _dot(a, b):
    return jnp.dot(a, b, preferred_element_type=f32)


def _bits(x, dt):
    return lax.bitcast_convert_type(x, dt)


def _recip(x):
    r = pl.reciprocal(x, approx=True)
    return r * (2.0 - x * r)


def _zero_after(v):
    return jnp.where(v < 0.0, 1.0, 0.0)


def _rowwise(x, w8, op):
    r, n = x.shape
    return op(x.reshape(r // 8, 8, n), w8[None]).reshape(r, n)


def _fold(x):
    n = x.shape[1] // T
    parts = [x[:, t * T:(t + 1) * T] for t in range(n)]
    nacc = 2 if n >= 4 else 1
    accs = parts[:nacc]
    for t in range(nacc, n):
        accs[t % nacc] = accs[t % nacc] + parts[t]
    return accs[0] if nacc == 1 else accs[0] + accs[1]


def _tile_lanes(v, n):
    return jnp.concatenate([v] * n, axis=1)


def _unpack_pair(w):
    lo = _bits(w << 16, f32)
    hi = _bits(w & jnp.uint32(0xFFFF0000), f32)
    return jnp.concatenate([lo, hi], axis=1).astype(bf)


def _top8(keys):
    keys = keys.reshape(keys.shape[0] // 8, 8, T)
    sub = lax.broadcasted_iota(i32, (8, T), 0)
    top = jnp.zeros((8, T), f32)
    for k in range(TOPK):
        mx = jnp.max(jnp.max(keys, axis=0), axis=0, keepdims=True)
        top = jnp.where(sub == k, mx, top)
        if k + 1 < TOPK:
            keys = jnp.where(keys == mx[None], 0.0, keys)
    return top


def _kernel(x_hbm, c_hbm, wq_hbm, wk_hbm, wv_hbm, wo_hbm, wr_hbm, wg_hbm, wu_hbm, wd_hbm, cv_hbm, wm_hbm,
            out_hbm,
            x_s, c_s, cp_s, h_s, hp_s, rq_s, rk_s, rv_s, q_s, k0_s, k_s, v_s, m_s, ctx_s,
            wo_s, wr_s, wg_s, wd_s, wt_s, cv_s, sc_s, wm_s, mod_s, att_s, h2_s, ob_s, out_s,
            key_s, fix_s, tk_s,
            sem_w, sem_c, sem_x, sem_m, sem_o, sem_b, *s_s):
    def w_copy(w_hbm, dst, sem_col, pair, slot):
        return pltpu.make_async_copy(w_hbm.bitcast(u32).at[:, pair, :], dst.at[slot], sem_w.at[slot, sem_col])

    def step_copies(j, par):
        return [w_copy(wq_hbm, rq_s, 2, j + 1, 1 - par), w_copy(wv_hbm, rv_s, 1, j + 1, 1 - par),
                w_copy(wk_hbm, rk_s, 0, jnp.minimum(j + 2, NP - 1), par)]

    c_cp = [pltpu.make_async_copy(c_hbm.at[pl.ds(a, b - a)], c_s.at[pl.ds(a, b - a)], sem_c.at[i])
            for i, (a, b) in enumerate(CCH)]
    x_cp = [pltpu.make_async_copy(x_hbm.at[pl.ds(a, b - a)], x_s.at[pl.ds(a, b - a)], sem_x.at[i])
            for i, (a, b) in enumerate(XCH)]
    cv_cp = pltpu.make_async_copy(cv_hbm, cv_s, sem_m.at[0])
    wm0_cp = pltpu.make_async_copy(wm_hbm.at[:, pl.ds(0, 2 * M)], wm_s.at[:, pl.ds(0, 2 * M)], sem_m.at[1])
    late_cp = [pltpu.make_async_copy(wm_hbm.at[:, pl.ds(2 * M, 4 * M)], wm_s.at[:, pl.ds(2 * M, 4 * M)], sem_m.at[2]),
               pltpu.make_async_copy(wo_hbm, wo_s, sem_m.at[3]),
               pltpu.make_async_copy(wr_hbm, wr_s, sem_m.at[4]),
               pltpu.make_async_copy(wg_hbm, wg_s.at[pl.ds(0, F)], sem_m.at[5]),
               pltpu.make_async_copy(wu_hbm, wg_s.at[pl.ds(FP, F)], sem_m.at[6]),
               pltpu.make_async_copy(wd_hbm, wd_s.at[pl.ds(0, F)], sem_m.at[7])]

    def out_copy(r0, n, k):
        return pltpu.make_async_copy(out_s.at[pl.ds(r0, n)], out_hbm.at[pl.ds(r0, n)], sem_o.at[k])

    def fence():
        pl.semaphore_signal(sem_b, 1)
        pl.semaphore_wait(sem_b, 1)

    def urgent(z, par=None):
        src = 0 if par is None else 1 - par
        dst = 0 if par is None else par
        for _ in range(NURG):
            tk_s[dst, 0:8, 0:T] = z.astype(bf)
            z = tk_s[src, 0:8, 0:T].astype(f32)
        return z

    def proj(lhs, w, dst, a, b):
        y = _dot(lhs, w)
        dst[0, a:b, :] = y[:, 0:D].astype(bf)
        dst[1, a:b, :] = y[:, D:2 * D].astype(bf)

    def c_rows(a, b):
        return pltpu.bitcast(cp_s[a // 2:b // 2, :], bf)

    lane = lax.broadcasted_iota(i32, (HS, T), 1)
    srow = lax.broadcasted_iota(i32, (HS, T), 0)
    diag = lane <= srow + HS
    half = [lane < HS, lane >= HS]
    first = [lane <= srow, jnp.logical_and(lane >= HS, lane - HS <= srow)]

    def q_rows(e, strips):
        return jnp.concatenate([q_s[e, HS * u:HS * (u + 1), :] for u in strips], axis=0)

    def left_scores(strips, kref):
        st = [lax.dot_general(kref[e, 0:HS, :], q_rows(e, strips), NT, preferred_element_type=f32) for e in range(2)]
        return jnp.concatenate(st, axis=0).T

    def qk(e, strips, kref, left=None):
        off = HS * (1 - strips[0] % 2)
        n0 = (strips[0] + 1) // 2
        q = q_rows(e, strips)
        parts = [[] for _ in strips]
        if n0 > 0:
            s = lax.dot_general(q, kref[e, off:off + n0 * T, :], NT, preferred_element_type=f32)
            for k in range(len(strips)):
                parts[k] += [s[HS * k:HS * (k + 1), t * T:(t + 1) * T] for t in range(n0)]
        for k0 in range(1, len(strips)):
            t = n0 + k0 - 1
            s = lax.dot_general(q[HS * k0:], kref[e, off + t * T:off + (t + 1) * T, :], NT, preferred_element_type=f32)
            for k in range(k0, len(strips)):
                parts[k].append(s[HS * (k - k0):HS * (k - k0 + 1), :])
        for k, u in enumerate(strips):
            if parts[k]:
                parts[k][-1] = jnp.where(diag, parts[k][-1], NEG)
            if u % 2 == 0:
                parts[k].insert(0, jnp.where(first[e] if u == 0 else half[e], left[HS * k:HS * (k + 1), :], NEG))
            su = jnp.concatenate(parts[k], axis=1)
            s_s[e * NS + u][...] = su
            m_s[e, HS * u:HS * (u + 1), :] = jnp.broadcast_to(jnp.max(su, axis=1, keepdims=True), (HS, D))

    groups = [[8 * b + par + 2 * k for k in range(4)] for b in range(NS // 8 - 1, -1, -1) for par in (1, 0)]

    def scores(kref):
        lefts = {}
        for e in range(2):
            for g in groups:
                if g[0] % 2 and g[0] - 1 not in lefts:
                    lefts[g[0] - 1] = left_scores([u - 1 for u in g], kref)
                qk(e, g, kref, None if g[0] % 2 else lefts[g[0]])

    def softmax(tok):
        P = {}
        for e in range(2):
            for g in groups:
                for u in g:
                    P[(e, u)] = []
                    n = u // 2 + 1
                    prev = None
                    for rr in range(0, HS, 8):
                        r = HS * u + rr
                        m = m_s[e, r:r + 8, :] + tok
                        p = jnp.exp2(s_s[e * NS + u][rr:rr + 8, :] - _tile_lanes(m, n))
                        acc = _fold(p)
                        P[(e, u)].append((p, acc))
                        if n > PAR_N:
                            tok = _zero_after(acc)
                        elif prev is None:
                            prev = acc
                        else:
                            tok = _zero_after(acc + prev)
                            prev = None
        return P, tok

    def values(e, pair, P):
        for g in groups:
            n0 = g[0] // 2 + 1
            ps = [jnp.concatenate([x[0] for x in P[(e, u)]], axis=0) for u in g]

            def vt(t0, t1):
                if g[0] % 2:
                    return v_s[e, t0 * T:t1 * T, :]
                if t0 > 0:
                    return v_s[e, t0 * T - HS:t1 * T - HS, :]
                vl = [v_s[0, 0:HS, :], v_s[1, 0:HS, :]]
                return jnp.concatenate(vl + ([v_s[e, HS:t1 * T - HS, :]] if t1 > 1 else []), axis=0)

            ctx = _dot(jnp.concatenate([x[:, 0:n0 * T] for x in ps], axis=0).astype(bf), vt(0, n0))
            cs = [ctx[HS * k:HS * (k + 1)] for k in range(len(g))]
            for k0 in range(1, len(g)):
                t = n0 + k0 - 1
                c2 = _dot(jnp.concatenate([x[:, t * T:(t + 1) * T] for x in ps[k0:]], axis=0).astype(bf), vt(t, t + 1))
                for k in range(k0, len(g)):
                    cs[k] = cs[k] + c2[HS * (k - k0):HS * (k - k0 + 1)]
            for k, u in enumerate(g):
                l = jnp.sum(jnp.concatenate([x[1] for x in P[(e, u)]], axis=0), axis=1, keepdims=True)
                ctx_s[2 * pair + e, HS * u:HS * (u + 1), :] = (cs[k] * _recip(l)).astype(bf)

    def ln1(i, tok):
        starts = list(range(XCH[i][1] - 8, XCH[i][0] - 1, -8))
        nu = len(starts)
        mean, rinv = {}, {}
        for t in range(nu + 2 * LK):
            if t < nu:
                a = starts[t]
                s1 = _fold(x_s[a:a + 8, :].astype(f32)) + tok
                mean[t] = jnp.sum(s1, axis=1, keepdims=True) * (1.0 / M)
                tok = _zero_after(s1 * s1)
            u = t - LK
            if 0 <= u < nu:
                a = starts[u]
                xc = x_s[a:a + 8, :].astype(f32) - _tile_lanes(mean[u] + tok, M // T)
                s2 = _fold(xc * xc)
                rinv[u] = lax.rsqrt(jnp.sum(s2, axis=1, keepdims=True) * (1.0 / M) + EPS)
                tok = _zero_after(s2)
            u = t - 2 * LK
            if 0 <= u < nu:
                a = starts[u]
                xn = (x_s[a:a + 8, :].astype(f32) - mean[u]) * _tile_lanes(rinv[u] + tok, M // T)
                hv = xn * mod_s[:, 0:M] + mod_s[:, M:2 * M]
                h_s[a:a + 8, :] = hv.astype(bf)
                z = _fold(hv)
                tok = _zero_after(z * z)
        return urgent(tok)

    wk0_cp, wv0_cp, wq0_cp = w_copy(wk_hbm, rk_s, 0, 0, 0), w_copy(wv_hbm, rv_s, 1, 0, 0), w_copy(wq_hbm, rq_s, 2, 0, 0)
    wk1_cp = w_copy(wk_hbm, rk_s, 0, 1, 1)
    for cp in [cv_cp, wk0_cp, c_cp[0], wv0_cp, c_cp[1], wk1_cp, c_cp[2], wm0_cp, x_cp[0], wq0_cp] + x_cp[1:]:
        cp.start()
        fence()

    tok = jnp.zeros((8, T), f32)
    for w_, o_ in ((wg_s, 0), (wg_s, FP), (wd_s, 0)):
        w_[o_ + F:o_ + FP, :] = jnp.zeros((FP - F, M), bf)
    tk_s[...] = jnp.zeros(tk_s.shape, bf)
    cv_cp.wait()
    cvec = cv_s[...].astype(f32)
    silu_c = _rb(cvec * jax.nn.sigmoid(cvec))
    sc_s[...] = jnp.broadcast_to(silu_c, (T, M)).T
    wk0_cp.wait(); c_cp[0].wait(); wv0_cp.wait()
    wk0 = _unpack_pair(rk_s[0])
    wv0 = _unpack_pair(rv_s[0])

    def kv0(a, b):
        lhs = c_s[a:b, :]
        cp_s[a // 2:b // 2, :] = pltpu.bitcast(lhs, u32)
        proj(lhs, wk0, k0_s, a, b)
        proj(lhs, wv0, v_s, a, b)

    kv0(*CCH[0])
    c_cp[1].wait()
    kv0(*CCH[1])
    wk1_cp.wait()
    wk1 = _unpack_pair(rk_s[1])

    def k1(a, b):
        proj(c_s[a:b, :], wk1, k_s, a, b)

    k1(0, CCH[2][0])
    c_cp[2].wait()
    kv0(*CCH[2])
    k1(CCH[2][0], K1)
    wm0_cp.wait(); x_cp[0].wait()
    mod0 = _rb(_dot(jnp.broadcast_to(silu_c.astype(bf), (8, M)), wm_s[:, 0:2 * M]))
    mod_s[:, 0:M] = _rb(1.0 + mod0[:, M:2 * M]) * QSCALE
    mod_s[:, M:2 * M] = mod0[:, 0:M] * QSCALE
    k1(K1, K2)
    tok = ln1(0, tok)
    wq0_cp.wait(); x_cp[1].wait()
    wq0 = _unpack_pair(rq_s[0])

    def q0(i):
        lhs = h_s[i * TQ:(i + 1) * TQ, :]
        hp_s[i * TQ // 2:(i + 1) * TQ // 2, :] = pltpu.bitcast(lhs, u32)
        proj(lhs, wq0, q_s, i * TQ, (i + 1) * TQ)

    lefts = {}

    def qk0(e, i):
        if i not in lefts:
            lefts[i] = left_scores([4 * i, 4 * i + 2], k0_s)
        qk(e, [4 * i + 1, 4 * i + 3], k0_s)
        qk(e, [4 * i, 4 * i + 2], k0_s, lefts[i])

    tok = ln1(1, tok)
    q0(7); k1(K2, K2 + T); qk0(0, 7); q0(6); qk0(1, 7); k1(K2 + T, K2 + 2 * T)
    for cp in step_copies(0, 0):
        cp.start()
    late_cp[3].start()
    late_cp[4].start()
    for cp in late_cp[:3] + late_cp[5:]:
        cp.start(priority=1)
    x_cp[2].wait()
    tok = ln1(2, tok)
    qk0(0, 6); qk0(1, 6)
    q0(5)
    k1(K2 + 2 * T, K3)
    qk0(0, 5); q0(4); qk0(1, 5); qk0(0, 4); q0(3); qk0(1, 4); qk0(0, 3); q0(2)
    q0(1); qk0(0, 2); q0(0); qk0(1, 2)
    qk0(0, 1); qk0(1, 1); qk0(0, 0); qk0(1, 0); qk0(1, 3)
    k1(K3, S)

    def late_mod(tok):
        for _ in range(MDEL):
            tok = tok * tok
        cols = []
        for jt in range(4 * M // T):
            w = wm_s[:, 2 * M + jt * T:2 * M + (jt + 1) * T].astype(f32)
            acc = None
            for g in range(M // 8):
                t_ = (w[8 * g:8 * g + 8, :] + tok) * sc_s[8 * g:8 * g + 8, :]
                acc = t_ if acc is None else acc + t_
                if (g + 1) % MODG == 0:
                    tok = _zero_after(acc * acc)
            cols.append(jnp.broadcast_to(jnp.sum(acc, axis=0, keepdims=True), (8, T)))
        mod1 = _rb(jnp.concatenate(cols, axis=1))
        mod_s[:, 0:2 * M] = mod1[:, 0:2 * M]
        mod_s[:, 2 * M:3 * M] = _rb(1.0 + mod1[:, 2 * M:3 * M])
        mod_s[:, 3 * M:4 * M] = mod1[:, 3 * M:4 * M]
        mod_s[:, 4 * M:5 * M] = jnp.broadcast_to(wr_s[...].astype(f32).reshape(1, M), (8, M))
        return tok

    def step(j, tok, last):
        par = j & 1
        for cp in step_copies(j, par):
            cp.wait()
        P, tok = softmax(tok)
        if last:
            tok = late_mod(tok)
        wq = _unpack_pair(rq_s[1 - par])
        if not last:
            for cp in step_copies(j + 1, 1 - par):
                cp.start()
        for a in range(0, S, PC):
            proj(pltpu.bitcast(hp_s[a // 2:(a + PC) // 2, :], bf), wq, q_s, a, a + PC)

        wv = _unpack_pair(rv_s[1 - par])

        def vproj(lo, hi):
            for a in range(lo, hi, PC):
                proj(c_rows(a, a + PC), wv, v_s, a, a + PC)

        values(0, j, P)
        values(1, j, P)
        vproj(0, VS if last else S)
        scores(k_s)
        if last:
            vproj(VS, S)
        else:
            wt_s[j] = wg_s[pl.ds(pl.multiple_of(j * TQ, TQ), TQ), :].T
            wk = _unpack_pair(rk_s[par])
            for a in range(S - PC, -1, -PC):
                proj(c_rows(a, a + PC), wk, k_s, a, a + PC)
        return urgent(tok, None if last else par)

    late_cp[3].wait(); late_cp[4].wait()
    tok = lax.fori_loop(0, NP - 2, lambda j, t: step(j, t, False), tok)
    late_cp[0].wait(); late_cp[2].wait()
    tok = step(NP - 2, tok, True)

    for cp in late_cp[1:2] + late_cp[5:]:
        cp.wait()

    def oproj(r0, n, h0, h1):
        lhs = jnp.concatenate([ctx_s[h, pl.ds(r0, n), :] for h in range(h0, h1)], axis=1)
        return _dot(lhs, wo_s[h0 * D:h1 * D, :])

    P, tok = softmax(tok)
    att_s[...] = oproj(S - RB, RB, 0, H - OS)
    values(0, NP - 1, P)
    values(1, NP - 1, P)
    att_s[...] += oproj(S - RB, RB, H - OS, H)
    key_s[...] = urgent(tok)

    def finish(r0, n, att, top, tok, paced):
        ga, sb, cb1, gb, wr = [mod_s[:, k * M:(k + 1) * M] for k in range(5)]
        keys = [top]
        for a in range(0, n, FR):
            ra = pl.multiple_of(r0 + a, FR)
            x1 = x_s[pl.ds(ra, FR), :].astype(f32) + _rowwise(att[a:a + FR, :], ga, jnp.multiply)
            m = jnp.sum(x1, axis=1, keepdims=True) * (1.0 / M)
            if tok is not None:
                m = m + tok
            xc = x1 - m
            rinv = lax.rsqrt(jnp.sum(xc * xc, axis=1, keepdims=True) * (1.0 / M) + EPS)
            h2 = _rowwise(_rowwise(xc * rinv, cb1, jnp.multiply), sb, jnp.add)
            h2_s[pl.ds(ra, FR), :] = h2
            ob = x1 + _rowwise(h2, gb, jnp.multiply)
            ob_s[pl.ds(ra, FR), :] = ob
            out_s[pl.ds(ra, FR), :] = ob.astype(bf)
            r = jnp.sum(_rowwise(h2, wr, jnp.multiply), axis=1, keepdims=True) + 0.0
            if paced:
                tok = _zero_after(r * r)
            b = _bits(jnp.broadcast_to(r, (FR, T)), i32) >> 13
            o = jnp.where(b < 0, (KHALF - 1) - (b & (KHALF - 1)), b + KHALF)
            rws = lax.broadcasted_iota(i32, (FR, T), 0) + ra
            keys.append(_bits((o << 11) + (KOFF + S - 1 - rws), f32))
            if paced or a + FR == n:
                keys = [_top8(jnp.concatenate(keys, axis=0))]
        return keys[0], tok

    def oblock(t, carry):
        r1 = pl.multiple_of(S - RB - t * (RA + RB), 16)
        top, tok = finish(r1, RB, att_s, key_s[...], None, True)
        r2 = pl.multiple_of(r1 - RA, 16)
        top, tok = finish(r2, RA, oproj(r2, RA, 0, H), top, tok, True)
        key_s[...] = top
        out_copy(r2, RA + RB, t).start()
        att_s[...] = oproj(pl.multiple_of(r2 - RB, 16), RB, 0, H)
        return carry

    lax.fori_loop(0, NB, oblock, 0)
    key_s[...] = finish(0, RB, att_s, key_s[...], None, False)[0]
    out_copy(0, RB, NB).start()

    sel = _bits(key_s[...], i32)
    rowid = (S - 1) - (sel & (S - 1))
    idxs = [jnp.clip(rowid[k, 0], 0, S - 1) for k in range(TOPK)]
    xs = jnp.concatenate([h2_s[pl.ds(ix, 1), :] for ix in idxs], axis=0).astype(bf)
    g = _rb(_dot(xs, jnp.concatenate([wt_s[t] for t in range(NQ - 1)], axis=1)))
    g = _rb(g * jax.nn.sigmoid(g))
    u = _rb(_dot(xs, jnp.concatenate([wt_s[NQ - 1 + t] for t in range(NQ - 1)], axis=1)))
    y = _rb(_dot((g * u).astype(bf), wd_s[...]))
    o = (sel - KOFF) >> 11
    rsel = _bits((jnp.where(o >= KHALF, o - KHALF, 2 * KHALF - 1 - o) << 13) | 4096, f32)
    gate = _rb(jax.nn.sigmoid(_rb(rsel)))[:, 0:1]
    base = jnp.concatenate([ob_s[pl.ds(ix, 1), :] for ix in idxs], axis=0)
    new = base + mod_s[:, 3 * M:4 * M] * (y * gate)
    prev = None
    for k in range(TOPK):
        g0 = pl.multiple_of(jnp.clip(idxs[k] >> 3, 0, S // GR - 1) * GR, GR)
        ob_s[pl.ds(idxs[k], 1), :] = new[k:k + 1, :]
        fix_s[k] = ob_s[pl.ds(g0, GR), :].astype(bf)
        if prev is None:
            for t in range(NB):
                out_copy(S - (t + 1) * (RA + RB), RA + RB, t).wait()
            out_copy(0, RB, NB).wait()
        else:
            prev.wait()
        prev = pltpu.make_async_copy(fix_s.at[k], out_hbm.at[pl.ds(g0, GR)], sem_o.at[0])
        prev.start()
        fence()
    prev.wait()


@jax.jit
def pallas_adaLN_cond__compressed_kv_cla__moe_arch_mod__prompt_kernel(
        A_x, A_c_kv, A_w_q, A_w_uk, A_w_uv, A_w_o, B_x, B_w_r, B_w_gate, B_w_up, B_w_down, c, w_mod):
    V = pltpu.VMEM
    scratch = [
        V((S, M), bf), V((S, C), bf), V((S // 2, C), u32), V((S, M), bf), V((S // 2, M), u32),
        V((2, M, D), u32), V((2, C, D), u32), V((2, C, D), u32),
        V((2, S, D), bf), V((2, S, D), bf), V((2, S, D), bf), V((2, S, D), bf),
        V((2, S, D), f32), V((H, S, D), bf),
        V((H * D, M), bf), V((M,), bf), V((2 * FP, M), bf), V((FP, M), bf),
        V((NP - 2, M, TQ), bf),
        V((1, M), bf), V((M, T), f32), V((M, 6 * M), bf), V((8, 5 * M), f32),
        V((RB, M), f32), V((S, M), f32), V((S, M), f32), V((S, M), bf),
        V((8, T), f32), V((TOPK, GR, M), bf), V((2, 16, 2 * T), bf),
        pltpu.SemaphoreType.DMA((2, 3)), pltpu.SemaphoreType.DMA((len(CCH),)), pltpu.SemaphoreType.DMA((len(XCH),)),
        pltpu.SemaphoreType.DMA((8,)), pltpu.SemaphoreType.DMA((NB + 1,)), pltpu.SemaphoreType.REGULAR,
    ] + [V((HS, (u // 2 + 1) * T), f32) for _ in range(2) for u in range(NS)]
    out = pl.pallas_call(
        _kernel,
        in_specs=[pl.BlockSpec(memory_space=pltpu.HBM)] * 12,
        out_specs=pl.BlockSpec(memory_space=pltpu.HBM),
        out_shape=jax.ShapeDtypeStruct((S, M), bf),
        scratch_shapes=scratch,
        compiler_params=pltpu.CompilerParams(vmem_limit_bytes=120 * 1024 * 1024, disable_bounds_checks=True,
                                             disable_semaphore_checks=True),
    )(A_x.reshape(S, M), A_c_kv.reshape(S, C), A_w_q, A_w_uk, A_w_uv, A_w_o.reshape(H * D, M),
      B_w_r, B_w_gate.T, B_w_up.T, B_w_down, c, w_mod)
    return out.reshape(1, S, M)
```

```python
import jax
import jax.numpy as jnp
from jax import lax
import jax.experimental.pallas as pl
import jax.experimental.pallas.tpu as pltpu

S, M, C, H, D, F, TOPK = 2048, 640, 512, 32, 128, 1728, 8
NP = H // 2
T = 128
TQ = 256
NQ = S // TQ
HS = 64
NS = S // HS
RA, RB, NB = 256, 128, 5
FP = 1792
PC = 512
FR = 16
GR = 8
PAR_N = 6
LK = 8
NURG = 32
CCH = [(0, 256), (256, 768), (768, 2048)]
XCH = [(1792, 2048), (1536, 1792), (0, 1536)]
K1, K2, K3 = 896, 1536, 1920
VS = 1536
OS = 4
MODG = 8
MDEL = 1400
bf = jnp.bfloat16
f32 = jnp.float32
u32 = jnp.uint32
i32 = jnp.int32
NT = (((1,), (1,)), ((), ()))
EPS = 1e-5
QSCALE = D ** -0.5 * 1.4426950408889634
NEG = -1e30
KOFF = 0x10000000
KHALF = 1 << 18


def _rb(x):
    return x.astype(bf).astype(f32)


def _dot(a, b):
    return jnp.dot(a, b, preferred_element_type=f32)


def _bits(x, dt):
    return lax.bitcast_convert_type(x, dt)


def _recip(x):
    r = pl.reciprocal(x, approx=True)
    return r * (2.0 - x * r)


def _zero_after(v):
    return jnp.where(v < 0.0, 1.0, 0.0)


def _rowwise(x, w8, op):
    r, n = x.shape
    return op(x.reshape(r // 8, 8, n), w8[None]).reshape(r, n)


def _fold(x):
    n = x.shape[1] // T
    parts = [x[:, t * T:(t + 1) * T] for t in range(n)]
    nacc = 2 if n >= 4 else 1
    accs = parts[:nacc]
    for t in range(nacc, n):
        accs[t % nacc] = accs[t % nacc] + parts[t]
    return accs[0] if nacc == 1 else accs[0] + accs[1]


def _tile_lanes(v, n):
    return jnp.concatenate([v] * n, axis=1)


def _unpack_pair(w):
    lo = _bits(w << 16, f32)
    hi = _bits(w & jnp.uint32(0xFFFF0000), f32)
    return jnp.concatenate([lo, hi], axis=1).astype(bf)


def _top8(keys):
    keys = keys.reshape(keys.shape[0] // 8, 8, T)
    sub = lax.broadcasted_iota(i32, (8, T), 0)
    top = jnp.zeros((8, T), f32)
    for k in range(TOPK):
        mx = jnp.max(jnp.max(keys, axis=0), axis=0, keepdims=True)
        top = jnp.where(sub == k, mx, top)
        if k + 1 < TOPK:
            keys = jnp.where(keys == mx[None], 0.0, keys)
    return top


def _kernel(x_hbm, c_hbm, wq_hbm, wk_hbm, wv_hbm, wo_hbm, wr_hbm, wg_hbm, wu_hbm, wd_hbm, cv_hbm, wm_hbm,
            out_hbm,
            x_s, c_s, cp_s, h_s, hp_s, rq_s, rk_s, rv_s, q_s, k0_s, k_s, v_s, m_s, ctx_s,
            wo_s, wr_s, wg_s, wd_s, wt_s, cv_s, sc_s, wm_s, mod_s, att_s, h2_s, ob_s, out_s,
            key_s, fix_s, tk_s,
            sem_w, sem_c, sem_x, sem_m, sem_o, sem_b, *s_s):
    def w_copy(w_hbm, dst, sem_col, pair, slot):
        return pltpu.make_async_copy(w_hbm.bitcast(u32).at[:, pair, :], dst.at[slot], sem_w.at[slot, sem_col])

    def step_copies(j, par):
        return [w_copy(wq_hbm, rq_s, 2, j + 1, 1 - par), w_copy(wv_hbm, rv_s, 1, j + 1, 1 - par),
                w_copy(wk_hbm, rk_s, 0, jnp.minimum(j + 2, NP - 1), par)]

    c_cp = [pltpu.make_async_copy(c_hbm.at[pl.ds(a, b - a)], c_s.at[pl.ds(a, b - a)], sem_c.at[i])
            for i, (a, b) in enumerate(CCH)]
    x_cp = [pltpu.make_async_copy(x_hbm.at[pl.ds(a, b - a)], x_s.at[pl.ds(a, b - a)], sem_x.at[i])
            for i, (a, b) in enumerate(XCH)]
    cv_cp = pltpu.make_async_copy(cv_hbm, cv_s, sem_m.at[0])
    wm0_cp = pltpu.make_async_copy(wm_hbm.at[:, pl.ds(0, 2 * M)], wm_s.at[:, pl.ds(0, 2 * M)], sem_m.at[1])
    late_cp = [pltpu.make_async_copy(wm_hbm.at[:, pl.ds(2 * M, 4 * M)], wm_s.at[:, pl.ds(2 * M, 4 * M)], sem_m.at[2]),
               pltpu.make_async_copy(wo_hbm, wo_s, sem_m.at[3]),
               pltpu.make_async_copy(wr_hbm, wr_s, sem_m.at[4]),
               pltpu.make_async_copy(wg_hbm, wg_s.at[pl.ds(0, F)], sem_m.at[5]),
               pltpu.make_async_copy(wu_hbm, wg_s.at[pl.ds(FP, F)], sem_m.at[6]),
               pltpu.make_async_copy(wd_hbm, wd_s.at[pl.ds(0, F)], sem_m.at[7])]

    def out_copy(r0, n, k):
        return pltpu.make_async_copy(out_s.at[pl.ds(r0, n)], out_hbm.at[pl.ds(r0, n)], sem_o.at[k])

    def fence():
        pl.semaphore_signal(sem_b, 1)
        pl.semaphore_wait(sem_b, 1)

    def urgent(z, par=None):
        src = 0 if par is None else 1 - par
        dst = 0 if par is None else par
        for _ in range(NURG):
            tk_s[dst, 0:8, 0:T] = z.astype(bf)
            z = tk_s[src, 0:8, 0:T].astype(f32)
        return z

    def proj(lhs, w, dst, a, b):
        y = _dot(lhs, w)
        dst[0, a:b, :] = y[:, 0:D].astype(bf)
        dst[1, a:b, :] = y[:, D:2 * D].astype(bf)

    def c_rows(a, b):
        return pltpu.bitcast(cp_s[a // 2:b // 2, :], bf)

    lane = lax.broadcasted_iota(i32, (HS, T), 1)
    srow = lax.broadcasted_iota(i32, (HS, T), 0)
    diag = lane <= srow + HS
    half = [lane < HS, lane >= HS]
    first = [lane <= srow, jnp.logical_and(lane >= HS, lane - HS <= srow)]

    def q_rows(e, strips):
        return jnp.concatenate([q_s[e, HS * u:HS * (u + 1), :] for u in strips], axis=0)

    def left_scores(strips, kref):
        st = [lax.dot_general(kref[e, 0:HS, :], q_rows(e, strips), NT, preferred_element_type=f32) for e in range(2)]
        return jnp.concatenate(st, axis=0).T

    def qk(e, strips, kref, left=None):
        off = HS * (1 - strips[0] % 2)
        n0 = (strips[0] + 1) // 2
        q = q_rows(e, strips)
        parts = [[] for _ in strips]
        if n0 > 0:
            s = lax.dot_general(q, kref[e, off:off + n0 * T, :], NT, preferred_element_type=f32)
            for k in range(len(strips)):
                parts[k] += [s[HS * k:HS * (k + 1), t * T:(t + 1) * T] for t in range(n0)]
        for k0 in range(1, len(strips)):
            t = n0 + k0 - 1
            s = lax.dot_general(q[HS * k0:], kref[e, off + t * T:off + (t + 1) * T, :], NT, preferred_element_type=f32)
            for k in range(k0, len(strips)):
                parts[k].append(s[HS * (k - k0):HS * (k - k0 + 1), :])
        for k, u in enumerate(strips):
            if parts[k]:
                parts[k][-1] = jnp.where(diag, parts[k][-1], NEG)
            if u % 2 == 0:
                parts[k].insert(0, jnp.where(first[e] if u == 0 else half[e], left[HS * k:HS * (k + 1), :], NEG))
            su = jnp.concatenate(parts[k], axis=1)
            s_s[e * NS + u][...] = su
            m_s[e, HS * u:HS * (u + 1), :] = jnp.broadcast_to(jnp.max(su, axis=1, keepdims=True), (HS, D))

    groups = [[8 * b + par + 2 * k for k in range(4)] for b in range(NS // 8 - 1, -1, -1) for par in (1, 0)]

    def scores(kref):
        lefts = {}
        for e in range(2):
            for g in groups:
                if g[0] % 2 and g[0] - 1 not in lefts:
                    lefts[g[0] - 1] = left_scores([u - 1 for u in g], kref)
                qk(e, g, kref, None if g[0] % 2 else lefts[g[0]])

    def softmax(tok):
        P = {}
        for e in range(2):
            for g in groups:
                for u in g:
                    P[(e, u)] = []
                    n = u // 2 + 1
                    prev = None
                    for rr in range(0, HS, 8):
                        r = HS * u + rr
                        m = m_s[e, r:r + 8, :] + tok
                        p = jnp.exp2(s_s[e * NS + u][rr:rr + 8, :] - _tile_lanes(m, n))
                        acc = _fold(p)
                        P[(e, u)].append((p, acc))
                        if n > PAR_N:
                            tok = _zero_after(acc)
                        elif prev is None:
                            prev = acc
                        else:
                            tok = _zero_after(acc + prev)
                            prev = None
        return P, tok

    def values(e, pair, P):
        for g in groups:
            n0 = g[0] // 2 + 1
            ps = [jnp.concatenate([x[0] for x in P[(e, u)]], axis=0) for u in g]

            def vt(t0, t1):
                if g[0] % 2:
                    return v_s[e, t0 * T:t1 * T, :]
                if t0 > 0:
                    return v_s[e, t0 * T - HS:t1 * T - HS, :]
                vl = [v_s[0, 0:HS, :], v_s[1, 0:HS, :]]
                return jnp.concatenate(vl + ([v_s[e, HS:t1 * T - HS, :]] if t1 > 1 else []), axis=0)

            ctx = _dot(jnp.concatenate([x[:, 0:n0 * T] for x in ps], axis=0).astype(bf), vt(0, n0))
            cs = [ctx[HS * k:HS * (k + 1)] for k in range(len(g))]
            for k0 in range(1, len(g)):
                t = n0 + k0 - 1
                c2 = _dot(jnp.concatenate([x[:, t * T:(t + 1) * T] for x in ps[k0:]], axis=0).astype(bf), vt(t, t + 1))
                for k in range(k0, len(g)):
                    cs[k] = cs[k] + c2[HS * (k - k0):HS * (k - k0 + 1)]
            for k, u in enumerate(g):
                l = jnp.sum(jnp.concatenate([x[1] for x in P[(e, u)]], axis=0), axis=1, keepdims=True)
                ctx_s[2 * pair + e, HS * u:HS * (u + 1), :] = (cs[k] * _recip(l)).astype(bf)

    def ln1(i, tok):
        starts = list(range(XCH[i][1] - 8, XCH[i][0] - 1, -8))
        nu = len(starts)
        mean, rinv = {}, {}
        for t in range(nu + 2 * LK):
            if t < nu:
                a = starts[t]
                s1 = _fold(x_s[a:a + 8, :].astype(f32)) + tok
                mean[t] = jnp.sum(s1, axis=1, keepdims=True) * (1.0 / M)
                tok = _zero_after(s1 * s1)
            u = t - LK
            if 0 <= u < nu:
                a = starts[u]
                xc = x_s[a:a + 8, :].astype(f32) - _tile_lanes(mean[u] + tok, M // T)
                s2 = _fold(xc * xc)
                rinv[u] = lax.rsqrt(jnp.sum(s2, axis=1, keepdims=True) * (1.0 / M) + EPS)
                tok = _zero_after(s2)
            u = t - 2 * LK
            if 0 <= u < nu:
                a = starts[u]
                xn = (x_s[a:a + 8, :].astype(f32) - mean[u]) * _tile_lanes(rinv[u] + tok, M // T)
                hv = xn * mod_s[:, 0:M] + mod_s[:, M:2 * M]
                h_s[a:a + 8, :] = hv.astype(bf)
                z = _fold(hv)
                tok = _zero_after(z * z)
        return urgent(tok)

    wk0_cp, wv0_cp, wq0_cp = w_copy(wk_hbm, rk_s, 0, 0, 0), w_copy(wv_hbm, rv_s, 1, 0, 0), w_copy(wq_hbm, rq_s, 2, 0, 0)
    wk1_cp = w_copy(wk_hbm, rk_s, 0, 1, 1)
    for cp in [cv_cp, wk0_cp, c_cp[0], wv0_cp, c_cp[1], wk1_cp, c_cp[2], wm0_cp, x_cp[0], wq0_cp] + x_cp[1:] + late_cp[3:5]:
        cp.start()
        fence()

    tok = jnp.zeros((8, T), f32)
    for w_, o_ in ((wg_s, 0), (wg_s, FP), (wd_s, 0)):
        w_[o_ + F:o_ + FP, :] = jnp.zeros((FP - F, M), bf)
    tk_s[...] = jnp.zeros(tk_s.shape, bf)
    cv_cp.wait()
    cvec = cv_s[...].astype(f32)
    silu_c = _rb(cvec * jax.nn.sigmoid(cvec))
    sc_s[...] = jnp.broadcast_to(silu_c, (T, M)).T
    wk0_cp.wait(); c_cp[0].wait(); wv0_cp.wait()
    wk0 = _unpack_pair(rk_s[0])
    wv0 = _unpack_pair(rv_s[0])

    def kv0(a, b):
        lhs = c_s[a:b, :]
        cp_s[a // 2:b // 2, :] = pltpu.bitcast(lhs, u32)
        proj(lhs, wk0, k0_s, a, b)
        proj(lhs, wv0, v_s, a, b)

    kv0(*CCH[0])
    c_cp[1].wait()
    kv0(*CCH[1])
    wk1_cp.wait()
    wk1 = _unpack_pair(rk_s[1])

    def k1(a, b):
        proj(c_s[a:b, :], wk1, k_s, a, b)

    k1(0, CCH[2][0])
    c_cp[2].wait()
    kv0(*CCH[2])
    k1(CCH[2][0], K1)
    wm0_cp.wait(); x_cp[0].wait()
    mod0 = _rb(_dot(jnp.broadcast_to(silu_c.astype(bf), (8, M)), wm_s[:, 0:2 * M]))
    mod_s[:, 0:M] = _rb(1.0 + mod0[:, M:2 * M]) * QSCALE
    mod_s[:, M:2 * M] = mod0[:, 0:M] * QSCALE
    k1(K1, K2)
    tok = ln1(0, tok)
    wq0_cp.wait(); x_cp[1].wait()
    wq0 = _unpack_pair(rq_s[0])

    def q0(i):
        lhs = h_s[i * TQ:(i + 1) * TQ, :]
        hp_s[i * TQ // 2:(i + 1) * TQ // 2, :] = pltpu.bitcast(lhs, u32)
        proj(lhs, wq0, q_s, i * TQ, (i + 1) * TQ)

    lefts = {}

    def qk0(e, i):
        if i not in lefts:
            lefts[i] = left_scores([4 * i, 4 * i + 2], k0_s)
        qk(e, [4 * i + 1, 4 * i + 3], k0_s)
        qk(e, [4 * i, 4 * i + 2], k0_s, lefts[i])

    tok = ln1(1, tok)
    q0(7); k1(K2, K2 + T); qk0(0, 7); q0(6); qk0(1, 7); k1(K2 + T, K2 + 2 * T)
    for cp in step_copies(0, 0):
        cp.start()
    for cp in late_cp[:3] + late_cp[5:]:
        cp.start(priority=1)
    x_cp[2].wait()
    tok = ln1(2, tok)
    qk0(0, 6); qk0(1, 6)
    q0(5)
    k1(K2 + 2 * T, K3)
    qk0(0, 5); q0(4); qk0(1, 5); qk0(0, 4); q0(3); qk0(1, 4); qk0(0, 3); q0(2)
    q0(1); qk0(0, 2); q0(0); qk0(1, 2)
    qk0(0, 1); qk0(1, 1); qk0(0, 0); qk0(1, 0); qk0(1, 3)
    k1(K3, S)

    def late_mod(tok):
        for _ in range(MDEL):
            tok = tok * tok
        cols = []
        for jt in range(4 * M // T):
            w = wm_s[:, 2 * M + jt * T:2 * M + (jt + 1) * T].astype(f32)
            acc = None
            for g in range(M // 8):
                t_ = (w[8 * g:8 * g + 8, :] + tok) * sc_s[8 * g:8 * g + 8, :]
                acc = t_ if acc is None else acc + t_
                if (g + 1) % MODG == 0:
                    tok = _zero_after(acc * acc)
            cols.append(jnp.broadcast_to(jnp.sum(acc, axis=0, keepdims=True), (8, T)))
        mod1 = _rb(jnp.concatenate(cols, axis=1))
        mod_s[:, 0:2 * M] = mod1[:, 0:2 * M]
        mod_s[:, 2 * M:3 * M] = _rb(1.0 + mod1[:, 2 * M:3 * M])
        mod_s[:, 3 * M:4 * M] = mod1[:, 3 * M:4 * M]
        mod_s[:, 4 * M:5 * M] = jnp.broadcast_to(wr_s[...].astype(f32).reshape(1, M), (8, M))
        return tok

    def step(j, tok, last):
        par = j & 1
        for cp in step_copies(j, par):
            cp.wait()
        P, tok = softmax(tok)
        if last:
            tok = late_mod(tok)
        wq = _unpack_pair(rq_s[1 - par])
        if not last:
            for cp in step_copies(j + 1, 1 - par):
                cp.start()
        for a in range(0, S, PC):
            proj(pltpu.bitcast(hp_s[a // 2:(a + PC) // 2, :], bf), wq, q_s, a, a + PC)

        wv = _unpack_pair(rv_s[1 - par])

        def vproj(lo, hi):
            for a in range(lo, hi, PC):
                proj(c_rows(a, a + PC), wv, v_s, a, a + PC)

        values(0, j, P)
        values(1, j, P)
        vproj(0, VS if last else S)
        scores(k_s)
        if last:
            vproj(VS, S)
        else:
            wt_s[j] = wg_s[pl.ds(pl.multiple_of(j * TQ, TQ), TQ), :].T
            wk = _unpack_pair(rk_s[par])
            for a in range(S - PC, -1, -PC):
                proj(c_rows(a, a + PC), wk, k_s, a, a + PC)
        return urgent(tok, None if last else par)

    late_cp[3].wait(); late_cp[4].wait()
    tok = lax.fori_loop(0, NP - 2, lambda j, t: step(j, t, False), tok)
    late_cp[0].wait(); late_cp[2].wait()
    tok = step(NP - 2, tok, True)

    for cp in late_cp[1:2] + late_cp[5:]:
        cp.wait()

    def oproj(r0, n, h0, h1):
        lhs = jnp.concatenate([ctx_s[h, pl.ds(r0, n), :] for h in range(h0, h1)], axis=1)
        return _dot(lhs, wo_s[h0 * D:h1 * D, :])

    P, tok = softmax(tok)
    att_s[...] = oproj(S - RB, RB, 0, H - OS)
    values(0, NP - 1, P)
    values(1, NP - 1, P)
    att_s[...] += oproj(S - RB, RB, H - OS, H)
    key_s[...] = urgent(tok)

    def finish(r0, n, att, top, tok, paced):
        ga, sb, cb1, gb, wr = [mod_s[:, k * M:(k + 1) * M] for k in range(5)]
        keys = [top]
        for a in range(0, n, FR):
            ra = pl.multiple_of(r0 + a, FR)
            x1 = x_s[pl.ds(ra, FR), :].astype(f32) + _rowwise(att[a:a + FR, :], ga, jnp.multiply)
            m = jnp.sum(x1, axis=1, keepdims=True) * (1.0 / M)
            if tok is not None:
                m = m + tok
            xc = x1 - m
            rinv = lax.rsqrt(jnp.sum(xc * xc, axis=1, keepdims=True) * (1.0 / M) + EPS)
            h2 = _rowwise(_rowwise(xc * rinv, cb1, jnp.multiply), sb, jnp.add)
            h2_s[pl.ds(ra, FR), :] = h2
            ob = x1 + _rowwise(h2, gb, jnp.multiply)
            ob_s[pl.ds(ra, FR), :] = ob
            out_s[pl.ds(ra, FR), :] = ob.astype(bf)
            if paced:
                r = jnp.sum(_rowwise(h2, wr, jnp.multiply), axis=1, keepdims=True) + 0.0
                tok = _zero_after(r * r)
            else:
                r = jnp.sum(_rowwise(xc, cb1 * wr, jnp.multiply), axis=1, keepdims=True) * rinv
                r = _rowwise(r, jnp.sum(sb * wr, axis=1, keepdims=True), jnp.add) + 0.0
            b = _bits(jnp.broadcast_to(r, (FR, T)), i32) >> 13
            o = jnp.where(b < 0, (KHALF - 1) - (b & (KHALF - 1)), b + KHALF)
            rws = lax.broadcasted_iota(i32, (FR, T), 0) + ra
            keys.append(_bits((o << 11) + (KOFF + S - 1 - rws), f32))
            if paced or a + FR == n:
                keys = [_top8(jnp.concatenate(keys, axis=0))]
        return keys[0], tok

    def oblock(t, carry):
        r1 = pl.multiple_of(S - RB - t * (RA + RB), 16)
        top, tok = finish(r1, RB, att_s, key_s[...], None, True)
        r2 = pl.multiple_of(r1 - RA, 16)
        top, tok = finish(r2, RA, oproj(r2, RA, 0, H), top, tok, True)
        key_s[...] = top
        out_copy(r2, RA + RB, t).start()
        att_s[...] = oproj(pl.multiple_of(r2 - RB, 16), RB, 0, H)
        return carry

    lax.fori_loop(0, NB, oblock, 0)
    key_s[...] = finish(0, RB, att_s, key_s[...], None, False)[0]
    out_copy(0, RB, NB).start()

    sel = _bits(key_s[...], i32)
    rowid = (S - 1) - (sel & (S - 1))
    idxs = [jnp.clip(rowid[k, 0], 0, S - 1) for k in range(TOPK)]
    xs = jnp.concatenate([h2_s[pl.ds(ix, 1), :] for ix in idxs], axis=0).astype(bf)
    g = _rb(_dot(xs, jnp.concatenate([wt_s[t] for t in range(NQ - 1)], axis=1)))
    g = _rb(g * jax.nn.sigmoid(g))
    u = _rb(_dot(xs, jnp.concatenate([wt_s[NQ - 1 + t] for t in range(NQ - 1)], axis=1)))
    y = _rb(_dot((g * u).astype(bf), wd_s[...]))
    o = (sel - KOFF) >> 11
    rsel = _bits((jnp.where(o >= KHALF, o - KHALF, 2 * KHALF - 1 - o) << 13) | 4096, f32)
    gate = _rb(jax.nn.sigmoid(_rb(rsel)))[:, 0:1]
    base = jnp.concatenate([ob_s[pl.ds(ix, 1), :] for ix in idxs], axis=0)
    new = base + mod_s[:, 3 * M:4 * M] * (y * gate)
    prev = None
    for k in range(TOPK):
        g0 = pl.multiple_of(jnp.clip(idxs[k] >> 3, 0, S // GR - 1) * GR, GR)
        ob_s[pl.ds(idxs[k], 1), :] = new[k:k + 1, :]
        fix_s[k] = ob_s[pl.ds(g0, GR), :].astype(bf)
        if prev is None:
            for t in range(NB):
                out_copy(S - (t + 1) * (RA + RB), RA + RB, t).wait()
            out_copy(0, RB, NB).wait()
        else:
            prev.wait()
        prev = pltpu.make_async_copy(fix_s.at[k], out_hbm.at[pl.ds(g0, GR)], sem_o.at[0])
        prev.start()
        fence()
    prev.wait()


@jax.jit
def pallas_adaLN_cond__compressed_kv_cla__moe_arch_mod__prompt_kernel(
        A_x, A_c_kv, A_w_q, A_w_uk, A_w_uv, A_w_o, B_x, B_w_r, B_w_gate, B_w_up, B_w_down, c, w_mod):
    V = pltpu.VMEM
    scratch = [
        V((S, M), bf), V((S, C), bf), V((S // 2, C), u32), V((S, M), bf), V((S // 2, M), u32),
        V((2, M, D), u32), V((2, C, D), u32), V((2, C, D), u32),
        V((2, S, D), bf), V((2, S, D), bf), V((2, S, D), bf), V((2, S, D), bf),
        V((2, S, D), f32), V((H, S, D), bf),
        V((H * D, M), bf), V((M,), bf), V((2 * FP, M), bf), V((FP, M), bf),
        V((NP - 2, M, TQ), bf),
        V((1, M), bf), V((M, T), f32), V((M, 6 * M), bf), V((8, 5 * M), f32),
        V((RB, M), f32), V((S, M), f32), V((S, M), f32), V((S, M), bf),
        V((8, T), f32), V((TOPK, GR, M), bf), V((2, 16, 2 * T), bf),
        pltpu.SemaphoreType.DMA((2, 3)), pltpu.SemaphoreType.DMA((len(CCH),)), pltpu.SemaphoreType.DMA((len(XCH),)),
        pltpu.SemaphoreType.DMA((8,)), pltpu.SemaphoreType.DMA((NB + 1,)), pltpu.SemaphoreType.REGULAR,
    ] + [V((HS, (u // 2 + 1) * T), f32) for _ in range(2) for u in range(NS)]
    out = pl.pallas_call(
        _kernel,
        in_specs=[pl.BlockSpec(memory_space=pltpu.HBM)] * 12,
        out_specs=pl.BlockSpec(memory_space=pltpu.HBM),
        out_shape=jax.ShapeDtypeStruct((S, M), bf),
        scratch_shapes=scratch,
        compiler_params=pltpu.CompilerParams(vmem_limit_bytes=120 * 1024 * 1024, disable_bounds_checks=True,
                                             disable_semaphore_checks=True),
    )(A_x.reshape(S, M), A_c_kv.reshape(S, C), A_w_q, A_w_uk, A_w_uv, A_w_o.reshape(H * D, M),
      B_w_r, B_w_gate.T, B_w_up.T, B_w_down, c, w_mod)
    return out.reshape(1, S, M)
```
